```python
import jax
import jax.numpy as jnp

def _softmax(x, axis=-1):
    return jax.nn.softmax(x, axis=axis)
def _gelu(x):
    return jax.nn.gelu(x, approximate=True)
def _silu(x):
    return jax.nn.silu(x)
def _sigmoid(x):
    return jax.nn.sigmoid(x)
def _layernorm(x, axis=-1, eps=1e-5):
    m = jnp.mean(x, axis=axis, keepdims=True)
    v = jnp.var(x, axis=axis, keepdims=True)
    return (x - m) / jnp.sqrt(v + eps)
def _scatter_add(tgt, idx, src, axis=0):
    return tgt.at[idx].add(src)
def _segment_sum(src, seg, n):
    return jax.ops.segment_sum(src, seg, n)
class _Rng:
    def __init__(self, key):
        self._k = key
    def _next(self):
        self._k, sub = jax.random.split(self._k)
        return sub
    def normal(self, shape):
        return jax.random.normal(self._next(), shape, dtype=jnp.bfloat16)
    def randint(self, lo, hi, shape):
        return jax.random.randint(self._next(), shape, lo, hi, dtype=jnp.int32)
    def uniform(self, shape, lo=0.0, hi=1.0):
        return jax.random.uniform(self._next(), shape, jnp.bfloat16, lo, hi)
    def permutation(self, n):
        return jax.random.permutation(self._next(), n)


kernel_name = 'standalone__instancenorm__prompt'

def setup_inputs():
    _rng = _Rng(jax.random.key(int.from_bytes(__import__("os").urandom(4), "little")))
    _w = (lambda a: (lambda t: t.astype(jnp.bfloat16) if jnp.issubdtype(t.dtype, jnp.floating) else t)(jnp.asarray(a)))
    B, C, H, W = 2, 1024, 2048, 32
    return {
        "x": _w((lambda *s: _rng.normal(s) * 0.05)(B, C, H, W)),
        "g": _w((lambda *s: _rng.normal(s) * 0.05)(C) + 1.0),
        "b": _w((lambda *s: _rng.normal(s) * 0.05)(C)),
    }

def reference(x, g, b):
    mu = x.mean(axis=(-2, -1), keepdims=True)
    var = ((x - mu) * (x - mu)).mean(axis=(-2, -1), keepdims=True)
    xhat = (x - mu) / jnp.sqrt(var + 1e-5)
    return xhat * g.reshape(1, -1, 1, 1) + b.reshape(1, -1, 1, 1)
```

```python
import jax
import jax.numpy as jnp
from jax import lax
import jax.experimental.pallas as pl
import jax.experimental.pallas.tpu as pltpu

_F32 = jnp.float32
_EPS = 1e-5

_NA = 8
_ST = 8
_WL = 1024
_LC = 512
_RDEPTH = 8
_EARLY = 4
_NCHUNK = 4


def _normalize_group(buf, j, gs, bs):
    w, h = buf.shape[-2:]
    inv_n = 1.0 / (w * h)
    nl = h // _LC
    mus = []
    for g in range(_NA):
        acc = None
        for l in range(nl):
            v = buf[j, g, :, pl.ds(l * _LC, _LC)].astype(_F32)
            acc = v if acc is None else acc + v
        mus.append(jnp.sum(acc, keepdims=True) * inv_n)
    scales = []
    for g in range(_NA):
        acc = None
        for l in range(nl):
            d = buf[j, g, :, pl.ds(l * _LC, _LC)].astype(_F32) - mus[g]
            d = d * d
            acc = d if acc is None else acc + d
        var = jnp.sum(acc, keepdims=True) * inv_n
        scales.append(gs[g] * lax.rsqrt(var + _EPS))
    for g in range(_NA):
        shift = bs[g] - mus[g] * scales[g]
        for l in range(nl):
            v = buf[j, g, :, pl.ds(l * _LC, _LC)].astype(_F32)
            buf[j, g, :, pl.ds(l * _LC, _LC)] = (v * scales[g] + shift).astype(buf.dtype)


def _kernel(x_hbm, g_hbm, b_hbm, o_hbm, buf, gb_v, gb_f, gb_s, rsem, wsem, gsem):
    _, _, w, h = x_hbm.shape
    c_total = g_hbm.shape[0] * g_hbm.shape[1]
    nsub = buf.shape[0]

    def loc(k):
        return (k // _ST) * _NA, k % _ST

    def rd(k, j):
        a0, r = loc(k)
        return pltpu.make_async_copy(x_hbm.at[pl.ds(a0, _NA), r], buf.at[j], rsem.at[j])

    def wr_start(k, j):
        a0, r = loc(k)
        for q in range(w // 8):
            for p in range(h // _WL):
                rows = pl.ds(q * 8, 8)
                cols = pl.ds(p * _WL, _WL)
                pltpu.make_async_copy(
                    buf.at[j, :, rows, cols],
                    o_hbm.at[pl.ds(a0, _NA), r, rows, cols],
                    wsem.at[j],
                ).start()

    def wr_wait(j):
        pltpu.make_async_copy(buf.at[j], buf.at[j], wsem.at[j]).wait()

    def comp(k, j):
        a0, r = loc(k)
        cs = [((a0 + i) * _ST + r) % c_total for i in range(_NA)]
        gs = [gb_s[0, c // 128, c % 128] for c in cs]
        bs = [gb_s[1, c // 128, c % 128] for c in cs]
        _normalize_group(buf, j, gs, bs)

    for j in range(_RDEPTH):
        rd(j, j).start()

    cg = pltpu.make_async_copy(g_hbm, gb_v.at[0], gsem.at[0])
    cb = pltpu.make_async_copy(b_hbm, gb_v.at[1], gsem.at[1])
    cg.start()
    cb.start()
    cg.wait()
    cb.wait()
    gb_f[...] = gb_v[...].astype(_F32)
    cs_ = pltpu.make_async_copy(gb_f, gb_s, gsem.at[0])
    cs_.start()
    cs_.wait()

    for ci in range(_NCHUNK):
        base = ci * nsub

        def rbody(j, carry, base=base):
            rd(base + j, j).wait()

            @pl.when(j + _RDEPTH < nsub)
            def _():
                rd(base + j + _RDEPTH, j + _RDEPTH).start()

            comp(base + j, j)
            return carry

        lax.fori_loop(0, nsub - 1, rbody, 0)
        rd(base + nsub - 1, nsub - 1).wait()

        def ws(j, carry, base=base):
            wr_start(base + j, j)
            return carry

        lax.fori_loop(0, _EARLY, ws, 0)
        comp(base + nsub - 1, nsub - 1)
        lax.fori_loop(_EARLY, nsub, ws, 0)

        def ww(j, carry):
            wr_wait(j)
            return carry

        lax.fori_loop(0, nsub, ww, 0)
        if ci + 1 < _NCHUNK:
            for j in range(_RDEPTH):
                rd(base + nsub + j, j).start()


@jax.jit
def pallas_standalone__instancenorm__prompt_kernel(
    x: jax.Array,
    g: jax.Array,
    b: jax.Array,
):
    bsz, c, h, w = x.shape
    n = bsz * c
    nsub = n // (_NA * _NCHUNK)
    xt = jnp.transpose(x, (0, 1, 3, 2)).reshape(n // _ST, _ST, w, h)
    g2 = g.reshape(c // 128, 128)
    b2 = b.reshape(c // 128, 128)
    buf_bytes = nsub * _NA * w * h * x.dtype.itemsize
    out = pl.pallas_call(
        _kernel,
        in_specs=[pl.BlockSpec(memory_space=pl.ANY)] * 3,
        out_specs=pl.BlockSpec(memory_space=pl.ANY),
        out_shape=jax.ShapeDtypeStruct(xt.shape, x.dtype),
        scratch_shapes=[
            pltpu.VMEM((nsub, _NA, w, h), x.dtype),
            pltpu.VMEM((2, c // 128, 128), g.dtype),
            pltpu.VMEM((2, c // 128, 128), _F32),
            pltpu.SMEM((2, c // 128, 128), _F32),
            pltpu.SemaphoreType.DMA((nsub,)),
            pltpu.SemaphoreType.DMA((nsub,)),
            pltpu.SemaphoreType.DMA((2,)),
        ],
        compiler_params=pltpu.CompilerParams(vmem_limit_bytes=buf_bytes + (8 << 20)),
    )(xt, g2, b2)
    return jnp.transpose(out.reshape(bsz, c, w, h), (0, 1, 3, 2))
```

```python
import jax
import jax.numpy as jnp
from jax import lax
import jax.experimental.pallas as pl
import jax.experimental.pallas.tpu as pltpu

_F32 = jnp.float32
_EPS = 1e-5

_NA = 8
_LST = 3
_ST = 1 << _LST
_LC = 512
_AHEAD = 2
_RING = 4
_N0 = 1
_EARLY = 2
_PIPE = 4
_NCHUNK = 3


def _shr(x, k):
    if isinstance(x, int):
        return x >> k
    return lax.shift_right_logical(x, jnp.int32(k))


def _fold(v):
    parts = [v[:, l:l + 128] for l in range(0, v.shape[1], 128)]
    while len(parts) > 1:
        parts = [parts[i] + parts[i + 1] for i in range(0, len(parts), 2)]
    p = parts[0]
    p = p + pltpu.roll(p, 4, 0)
    p = p + pltpu.roll(p, 2, 0)
    p = p + pltpu.roll(p, 1, 0)
    return p


def _lanesum(p):
    return jnp.broadcast_to(jnp.sum(p, axis=1, keepdims=True), (8, 128))


def _slabs(buf):
    w, h = buf.shape[-2:]
    return [(pl.ds(q * 8, 8), pl.ds(l * _LC, _LC))
            for q in range(w // 8) for l in range(h // _LC)]


def _pass_sum(buf, i):
    acc = None
    for r, c in _slabs(buf):
        v = buf[i, r, c].astype(_F32)
        acc = v if acc is None else acc + v
    return _fold(acc)


def _pass_var(buf, i, mu):
    acc = None
    m = jnp.tile(mu, (1, _LC // 128))
    for r, c in _slabs(buf):
        d = buf[i, r, c].astype(_F32) - m
        d = d * d
        acc = d if acc is None else acc + d
    return _fold(acc)


def _pass_norm(buf, i, scale, shift):
    s = jnp.tile(scale, (1, _LC // 128))
    t = jnp.tile(shift, (1, _LC // 128))
    for r, c in _slabs(buf):
        v = buf[i, r, c].astype(_F32)
        buf[i, r, c] = (v * s + t).astype(buf.dtype)


def _make_kernel(chunks):
    def kernel(x_hbm, g_hbm, b_hbm, o_hbm, buf, gb_v, gb_f, gb_s, rsem, wsem, gsem):
        _, _, w, h = x_hbm.shape
        c_total = g_hbm.shape[0] * g_hbm.shape[1]
        inv_n = 1.0 / (w * h)
        dummy = buf.shape[0] - 1
        half = h // 2
        npc = (w // 8) * 2

        def loc(k):
            return _shr(k, _LST) * _NA, k & (_ST - 1)

        def rd_piece(kg, j, u):
            a0, r = loc(kg)
            rows = pl.ds(pl.multiple_of(_shr(u, 1) * 8, 8), 8)
            cols = pl.ds(pl.multiple_of((u & 1) * half, 128), half)
            sem = rsem.at[j & (_RING - 1)]
            pltpu.make_async_copy(
                x_hbm.at[pl.ds(a0 + _N0, _NA - _N0), r, rows, cols],
                buf.at[pl.ds(j * _NA + _N0, _NA - _N0), rows, cols],
                sem).start(priority=1)
            pltpu.make_async_copy(
                x_hbm.at[pl.ds(a0, _N0), r, rows, cols],
                buf.at[pl.ds(j * _NA, _N0), rows, cols],
                sem).start(priority=0)

        def rd_wait(j):
            grp = buf.at[pl.ds(j * _NA, _NA)]
            pltpu.make_async_copy(grp, grp, rsem.at[j & (_RING - 1)]).wait()

        def wr_start(kg, j):
            a0, r = loc(kg)
            for p in range(npc):
                rows = pl.ds((p // 2) * 8, 8)
                cols = pl.ds((p % 2) * half, half)
                pltpu.make_async_copy(
                    buf.at[pl.ds(j * _NA, _NA), rows, cols],
                    o_hbm.at[pl.ds(a0, _NA), r, rows, cols],
                    wsem.at[0]).start()

        def first_reads(kg0):
            def body(i, c):
                rd_piece(kg0 + _shr(i, 3), _shr(i, 3), i & 7)
                return c
            lax.fori_loop(0, _AHEAD * npc, body, 0)

        first_reads(0)

        cg = pltpu.make_async_copy(g_hbm, gb_v.at[0], gsem.at[0])
        cb = pltpu.make_async_copy(b_hbm, gb_v.at[1], gsem.at[1])
        cg.start()
        cb.start()
        buf[dummy] = jnp.zeros((w, h), buf.dtype)
        cg.wait()
        cb.wait()
        gb_f[...] = gb_v[...].astype(_F32)
        cs = pltpu.make_async_copy(gb_f, gb_s, gsem.at[0])
        cs.start()
        cs.wait()

        def chunk(kg0, ng, is_last, carry):
            n = ng * _NA

            def step(j, u, carry, head):
                p1, s1, p2, mu1, s2, mu2 = carry
                if head:
                    rd_piece(kg0 + j + _AHEAD, j + _AHEAD, u)
                ta = j * _NA + u
                t = ta - _PIPE
                tc = jnp.maximum(t, 0)
                a0, r = loc(kg0 + _shr(tc, 3))
                c = ((a0 + (tc & 7)) * _ST + r) & (c_total - 1)
                g = gb_s[0, _shr(c, 7), c & 127]
                b = gb_s[1, _shr(c, 7), c & 127]
                n_s1 = _lanesum(p1)
                n_s2 = _lanesum(p2)
                mu = s1 * inv_n
                scale = g * lax.rsqrt(s2 * inv_n + _EPS)
                shift = b - mu2 * scale
                if head:
                    ia, ib = ta, jnp.maximum(ta - 2, 0)
                    ic = jnp.where(t >= 0, t, dummy)
                else:
                    ia, ib, ic = jnp.minimum(ta, n - 1), jnp.minimum(ta - 2, n - 1), t
                n_p1 = _pass_sum(buf, ia)
                n_p2 = _pass_var(buf, ib, mu)
                _pass_norm(buf, ic, scale, shift)
                return n_p1, n_s1, n_p2, mu, n_s2, mu1

            def head_group(j, carry):
                rd_wait(j)
                return lax.fori_loop(0, _NA, lambda u, c: step(j, u, c, True), carry)

            def tail_group(j, carry):
                rd_wait(j)

                @pl.when(j == ng - 1)
                def _():
                    for jj in range(_EARLY):
                        wr_start(kg0 + jj, jj)

                nsteps = jnp.where(j == ng - 1, _NA + _PIPE, _NA)
                return lax.fori_loop(0, nsteps, lambda u, c: step(j, u, c, False), carry)

            carry = lax.fori_loop(0, ng - _AHEAD, head_group, carry)
            carry = lax.fori_loop(ng - _AHEAD, ng, tail_group, carry)

            def ws(j, c):
                wr_start(kg0 + j, j)
                return c

            lax.fori_loop(_EARLY, ng, ws, 0)
            used = buf.at[pl.ds(0, n)]
            pltpu.make_async_copy(used, used, wsem.at[0]).wait()
            if not is_last:
                first_reads(kg0 + ng)
            return carry

        carry = (gb_f[0],) * 6
        kg0 = 0
        for ci, ng in enumerate(chunks):
            carry = chunk(kg0, ng, ci == len(chunks) - 1, carry)
            kg0 += ng

    return kernel


@jax.jit
def pallas_standalone__instancenorm__prompt_kernel(
    x: jax.Array,
    g: jax.Array,
    b: jax.Array,
):
    bsz, c, h, w = x.shape
    n = bsz * c
    groups = n // _NA
    chunks = tuple(groups // _NCHUNK + (i < groups % _NCHUNK) for i in range(_NCHUNK))
    slots = max(chunks) * _NA + 1
    xt = jnp.transpose(x, (0, 1, 3, 2)).reshape(n // _ST, _ST, w, h)
    g2 = g.reshape(c // 128, 128)
    b2 = b.reshape(c // 128, 128)
    buf_bytes = slots * w * h * x.dtype.itemsize
    out = pl.pallas_call(
        _make_kernel(chunks),
        in_specs=[pl.BlockSpec(memory_space=pl.ANY)] * 3,
        out_specs=pl.BlockSpec(memory_space=pl.ANY),
        out_shape=jax.ShapeDtypeStruct(xt.shape, x.dtype),
        scratch_shapes=[
            pltpu.VMEM((slots, w, h), x.dtype),
            pltpu.VMEM((2, c // 128, 128), g.dtype),
            pltpu.VMEM((2, c // 128, 128), _F32),
            pltpu.SMEM((2, c // 128, 128), _F32),
            pltpu.SemaphoreType.DMA((_RING,)),
            pltpu.SemaphoreType.DMA((1,)),
            pltpu.SemaphoreType.DMA((2,)),
        ],
        compiler_params=pltpu.CompilerParams(vmem_limit_bytes=buf_bytes + (8 << 20)),
    )(xt, g2, b2)
    return jnp.transpose(out.reshape(bsz, c, w, h), (0, 1, 3, 2))
```

```python
import jax
import jax.numpy as jnp
from jax import lax
import jax.experimental.pallas as pl
import jax.experimental.pallas.tpu as pltpu

_F32 = jnp.float32
_EPS = 1e-5

_COLS = 8
_NA = 8
_N0 = 1
_FLIGHT = 8
_AHEAD = _NA - 1 + _FLIGHT
_WK = 6
_EARLY = 4
_RW = 4
_LC = 512
_PIPE = 4
_CHUNK = 96


def _shr(x, k):
    if isinstance(x, int):
        return x >> k
    return lax.shift_right_logical(x, jnp.int32(k))


def _fold(v):
    parts = [v[:, l:l + 128] for l in range(0, v.shape[1], 128)]
    while len(parts) > 1:
        parts = [parts[i] + parts[i + 1] for i in range(0, len(parts), 2)]
    p = parts[0]
    p = p + pltpu.roll(p, 4, 0)
    p = p + pltpu.roll(p, 2, 0)
    p = p + pltpu.roll(p, 1, 0)
    return p


def _lanesum(p):
    return jnp.broadcast_to(jnp.sum(p, axis=1, keepdims=True), (8, 128))


def _slabs(buf):
    w, h = buf.shape[-2:]
    return [(pl.ds(q * 8, 8), pl.ds(l * _LC, _LC))
            for q in range(w // 8) for l in range(h // _LC)]


def _pass_sum(buf, a, r):
    acc = None
    for s, c in _slabs(buf):
        v = buf[a, r, s, c].astype(_F32)
        acc = v if acc is None else acc + v
    return _fold(acc)


def _pass_var(buf, a, r, mu):
    acc = None
    m = jnp.tile(mu, (1, _LC // 128))
    for s, c in _slabs(buf):
        d = buf[a, r, s, c].astype(_F32) - m
        d = d * d
        acc = d if acc is None else acc + d
    return _fold(acc)


def _pass_norm(buf, a, r, scale, shift):
    sc = jnp.tile(scale, (1, _LC // 128))
    sh = jnp.tile(shift, (1, _LC // 128))
    for s, c in _slabs(buf):
        v = buf[a, r, s, c].astype(_F32)
        buf[a, r, s, c] = (v * sc + sh).astype(buf.dtype)


def _write_blocks(nrows):
    nb = -(-nrows // _WK)
    base, rem = divmod(nrows, nb)
    return [base + 1] * rem + [base] * (nb - rem)


def _kernel(x_hbm, g_hbm, b_hbm, o_hbm, buf, gb_v, gb_f, gb_s, rsem, wsem):
    rows_total, _, w, h = x_hbm.shape
    c_total = g_hbm.shape[0] * g_hbm.shape[1]
    inv_n = 1.0 / (w * h)
    dummy = buf.shape[0] - 1
    half = h // 2

    def group(i):
        j = _shr(i, 3)
        return _shr(j, 3) * _NA, j & (_COLS - 1)

    def inst(i):
        a0, r = group(i)
        return a0 + (i & (_NA - 1)), r

    def piece(u):
        if isinstance(u, int):
            return pl.ds((u >> 1) * 8, 8), pl.ds((u & 1) * half, half)
        return (pl.ds(pl.multiple_of(_shr(u, 1) * 8, 8), 8),
                pl.ds(pl.multiple_of((u & 1) * half, 128), half))

    def rd_start(row0, i):
        a0, r = group(i)
        s, c = piece(i & (_NA - 1))
        sem = rsem.at[i & (_FLIGHT - 1)]
        pltpu.make_async_copy(
            x_hbm.at[pl.ds(row0 + a0 + _N0, _NA - _N0), r, s, c],
            buf.at[pl.ds(a0 + _N0, _NA - _N0), r, s, c], sem).start(priority=1)
        pltpu.make_async_copy(
            x_hbm.at[pl.ds(row0 + a0, _N0), r, s, c],
            buf.at[pl.ds(a0, _N0), r, s, c], sem).start(priority=0)

    def rd_wait(i):
        a0, r = group(i)
        s, c = piece(i & (_NA - 1))
        v = buf.at[pl.ds(a0, _NA), r, s, c]
        pltpu.make_async_copy(v, v, rsem.at[i & (_FLIGHT - 1)]).wait()

    def wr_copy(row0, a0, k, r, p, sem):
        s, c = piece(p)
        return pltpu.make_async_copy(
            buf.at[pl.ds(a0, k), r, s, c],
            o_hbm.at[pl.ds(row0 + a0, k), r, s, c], sem)

    def wr_column(row0, a0, k, r, sem):
        for p in range(_NA):
            wr_copy(row0, a0, k, r, p, sem).start()

    def first_reads(row0):
        def body(i, c):
            rd_start(row0, i)
            return c
        lax.fori_loop(0, _FLIGHT, body, 0)

    def ramp(row0):
        def body(i, c):
            rd_wait(i)
            rd_start(row0, i + _FLIGHT)
            return c
        lax.fori_loop(0, _NA - 1, body, 0)

    first_reads(0)

    cg = pltpu.make_async_copy(g_hbm, gb_v.at[0], wsem.at[0])
    cb = pltpu.make_async_copy(b_hbm, gb_v.at[1], wsem.at[1])
    cg.start()
    cb.start()
    buf[dummy, 0] = jnp.zeros((w, h), buf.dtype)
    cg.wait()
    cb.wait()
    gb_f[...] = gb_v[...].astype(_F32)
    cs = pltpu.make_async_copy(gb_f, gb_s, wsem.at[2])
    cs.start()
    ramp(0)
    cs.wait()

    def chunk(row0, nrows, has_next, carry):
        n = nrows * _COLS

        def step(ta, carry, head):
            p1, s1, p2, mu1, s2, mu2 = carry
            if head:
                rd_wait(ta + _NA - 1)
                rd_start(row0, ta + _AHEAD)
            t = ta - _PIPE
            ac, rc = inst(jnp.maximum(t, 0))
            c = ((row0 + ac) * _COLS + rc) & (c_total - 1)
            g = gb_s[0, _shr(c, 7), c & 127]
            b = gb_s[1, _shr(c, 7), c & 127]
            n_s1 = _lanesum(p1)
            n_s2 = _lanesum(p2)
            mu = s1 * inv_n
            scale = g * lax.rsqrt(s2 * inv_n + _EPS)
            shift = b - mu2 * scale
            if head:
                aa, ra = inst(ta)
                ab, rb = inst(jnp.maximum(ta - 2, 0))
                ac = jnp.where(t >= 0, ac, dummy)
            else:
                aa, ra = inst(jnp.minimum(ta, n - 1))
                ab, rb = inst(jnp.minimum(ta - 2, n - 1))
            n_p1 = _pass_sum(buf, aa, ra)
            n_p2 = _pass_var(buf, ab, rb, mu)
            _pass_norm(buf, ac, rc, scale, shift)
            return n_p1, n_s1, n_p2, mu, n_s2, mu1

        nhead = n - _AHEAD
        carry = lax.fori_loop(0, nhead, lambda i, c: step(i, c, True), carry)
        for i in range(n - _FLIGHT, n - _RW):
            rd_wait(i)

        blocks = _write_blocks(nrows)
        for r in range(_EARLY):
            wr_column(row0, 0, blocks[0], r, wsem.at[0])
        for i in range(n - _RW, n):
            rd_wait(i)
        carry = lax.fori_loop(nhead, n + _PIPE, lambda i, c: step(i, c, False), carry)

        def columns(q0, q1, a_base, k, sem):
            def body(q, c):
                wr_column(row0, a_base + _shr(q, 3) * k, k, q & (_COLS - 1), sem)
                return c
            lax.fori_loop(q0, q1, body, 0)

        a_base, q0 = 0, _EARLY
        for k in sorted(set(blocks[:-1]), reverse=True):
            cnt = blocks[:-1].count(k)
            columns(q0, cnt * _COLS, a_base, k, wsem.at[0])
            a_base, q0 = a_base + cnt * k, 0
        kl = blocks[-1]
        columns(0, _COLS - 1, a_base, kl, wsem.at[1])
        last = [wr_copy(row0, a_base, kl, _COLS - 1, p, wsem.at[2 if p < _NA - 1 else 3])
                for p in range(_NA)]
        for cp in last:
            cp.start()
        v0 = buf.at[pl.ds(0, a_base)]
        pltpu.make_async_copy(v0, v0, wsem.at[0]).wait()
        v1 = buf.at[pl.ds(a_base, kl), pl.ds(0, _COLS - 1)]
        pltpu.make_async_copy(v1, v1, wsem.at[1]).wait()
        for cp in last[:-1]:
            cp.wait()
        if has_next:
            first_reads(row0 + nrows)
        last[-1].wait()
        if has_next:
            ramp(row0 + nrows)
        return carry

    carry = (gb_f[0],) * 6
    nfull = (rows_total - 1) // _CHUNK
    carry = lax.fori_loop(
        0, nfull, lambda ci, c: chunk(ci * _CHUNK, _CHUNK, True, c), carry)
    chunk(nfull * _CHUNK, rows_total - nfull * _CHUNK, False, carry)


@jax.jit
def pallas_standalone__instancenorm__prompt_kernel(
    x: jax.Array,
    g: jax.Array,
    b: jax.Array,
):
    bsz, c, h, w = x.shape
    rows = bsz * c // _COLS
    assert w == 32 and h % (2 * _LC) == 0 and c == 1024
    assert rows % _NA == 0 and (rows - 1) % _CHUNK + 1 >= 3 * _NA
    xt = jnp.transpose(x, (0, 1, 3, 2)).reshape(rows, _COLS, w, h)
    g2 = g.reshape(c // 128, 128)
    b2 = b.reshape(c // 128, 128)
    buf_bytes = (_CHUNK + 1) * _COLS * w * h * x.dtype.itemsize
    out = pl.pallas_call(
        _kernel,
        in_specs=[pl.BlockSpec(memory_space=pl.ANY)] * 3,
        out_specs=pl.BlockSpec(memory_space=pl.ANY),
        out_shape=jax.ShapeDtypeStruct(xt.shape, x.dtype),
        scratch_shapes=[
            pltpu.VMEM((_CHUNK + 1, _COLS, w, h), x.dtype),
            pltpu.VMEM((2, c // 128, 128), g.dtype),
            pltpu.VMEM((2, c // 128, 128), _F32),
            pltpu.SMEM((2, c // 128, 128), _F32),
            pltpu.SemaphoreType.DMA((_FLIGHT,)),
            pltpu.SemaphoreType.DMA((4,)),
        ],
        compiler_params=pltpu.CompilerParams(vmem_limit_bytes=buf_bytes + (8 << 20)),
    )(xt, g2, b2)
    return jnp.transpose(out.reshape(bsz, c, w, h), (0, 1, 3, 2))
```

```python
import jax
import jax.numpy as jnp
from jax import lax
import jax.experimental.pallas as pl
import jax.experimental.pallas.tpu as pltpu

_F32 = jnp.float32
_EPS = 1e-5

_COLS = 8
_NA = 16
_N0 = 2
_FLIGHT = 8
_AHEAD = _NA - 1 + _FLIGHT
_WK = 6
_EARLY = 5
_RW = 4
_LC = 512
_PIPE = 4
_CHUNK = 96


def _shr(x, k):
    if isinstance(x, int):
        return x >> k
    return lax.shift_right_logical(x, jnp.int32(k))


def _ds(start, size, align):
    if isinstance(start, int):
        return pl.ds(start, size)
    return pl.ds(pl.multiple_of(start, align), size)


def _fold(v):
    parts = [v[:, l:l + 128] for l in range(0, v.shape[1], 128)]
    while len(parts) > 1:
        parts = [parts[i] + parts[i + 1] for i in range(0, len(parts), 2)]
    p = parts[0]
    p = p + pltpu.roll(p, 4, 0)
    p = p + pltpu.roll(p, 2, 0)
    p = p + pltpu.roll(p, 1, 0)
    return p


def _lanesum(p):
    return jnp.broadcast_to(jnp.sum(p, axis=1, keepdims=True), (8, 128))


def _slabs(buf):
    w, h = buf.shape[-2:]
    return [(pl.ds(q * 8, 8), pl.ds(l * _LC, _LC))
            for q in range(w // 8) for l in range(h // _LC)]


def _pass_sum(buf, a, r):
    acc = None
    for s, c in _slabs(buf):
        v = buf[a, r, s, c].astype(_F32)
        acc = v if acc is None else acc + v
    return _fold(acc)


def _pass_center(buf, a, r, mu, dbuf, k):
    acc = None
    m = jnp.tile(mu, (1, _LC // 128))
    for s, c in _slabs(buf):
        d = buf[a, r, s, c].astype(_F32) - m
        dbuf[k, s, c] = d
        d = d * d
        acc = d if acc is None else acc + d
    return _fold(acc)


def _pass_norm(buf, a, r, scale, beta, dbuf, k):
    sc = jnp.tile(scale, (1, _LC // 128))
    for s, c in _slabs(buf):
        buf[a, r, s, c] = (dbuf[k, s, c] * sc + beta).astype(buf.dtype)


def _write_blocks(nrows):
    nb = -(-nrows // _WK)
    base, rem = divmod(nrows, nb)
    return [base + 1] * rem + [base] * (nb - rem)


def _kernel(x_hbm, g_hbm, b_hbm, o_hbm, buf, dbuf, gb_v, gb_f, gb_s, rsem, wsem):
    rows_total, _, w, h = x_hbm.shape
    c_total = g_hbm.shape[0] * g_hbm.shape[1]
    inv_n = 1.0 / (w * h)
    dummy = buf.shape[0] - 1
    rl = h // 4
    wl = h // 2

    def group(i):
        j = _shr(i, 4)
        return _shr(j, 3) * _NA, j & (_COLS - 1)

    def inst(i):
        a0, r = group(i)
        return a0 + (i & (_NA - 1)), r

    def rd_start(row0, i):
        a0, r = group(i)
        s = _ds((_shr(i, 2) & 3) * 8, 8, 8)
        sem = rsem.at[i & (_FLIGHT - 1)]
        for e, hi in ((0, True), (0, False), (1, False), (1, True)):
            c = _ds((i & 3) * rl + e * (rl // 2), rl // 2, 128)
            off, cnt = (0, _N0) if hi else (_N0, _NA - _N0)
            pltpu.make_async_copy(
                x_hbm.at[pl.ds(row0 + a0 + off, cnt), r, s, c],
                buf.at[pl.ds(a0 + off, cnt), r, s, c],
                sem).start(priority=0 if hi else 1)

    def rd_wait(i):
        a0, r = group(i)
        v = buf.at[pl.ds(a0, _NA), r,
                   _ds((_shr(i, 2) & 3) * 8, 8, 8), _ds((i & 3) * rl, rl, 128)]
        pltpu.make_async_copy(v, v, rsem.at[i & (_FLIGHT - 1)]).wait()

    def wr_copy(row0, a0, k, r, p, sem):
        s, c = pl.ds((p >> 1) * 8, 8), pl.ds((p & 1) * wl, wl)
        return pltpu.make_async_copy(
            buf.at[pl.ds(a0, k), r, s, c],
            o_hbm.at[pl.ds(row0 + a0, k), r, s, c], sem)

    def wr_column(row0, a0, k, r, sem):
        for p in range(8):
            wr_copy(row0, a0, k, r, p, sem).start()

    def first_reads(row0):
        for i in range(_FLIGHT):
            rd_start(row0, i)

    def ramp(row0):
        def body(i, c):
            rd_wait(i)
            rd_start(row0, i + _FLIGHT)
            return c
        lax.fori_loop(0, _NA - 1, body, 0)

    first_reads(0)

    cg = pltpu.make_async_copy(g_hbm, gb_v.at[0], wsem.at[0])
    cb = pltpu.make_async_copy(b_hbm, gb_v.at[1], wsem.at[1])
    cg.start()
    cb.start()
    dbuf[pl.ds(0, 2)] = jnp.zeros((2, w, h), _F32)
    cg.wait()
    cb.wait()
    gb_f[...] = gb_v[...].astype(_F32)
    cs = pltpu.make_async_copy(gb_f, gb_s, wsem.at[2])
    cs.start()
    ramp(0)
    cs.wait()

    def chunk(row0, nrows, has_next, carry):
        n = nrows * _COLS

        def step(ta, carry, head):
            p1, s1, p2, s2 = carry
            if head:
                rd_wait(ta + _NA - 1)
            t = ta - _PIPE
            ac, rc = inst(jnp.maximum(t, 0))
            ac = jnp.where(t >= 0, ac, dummy)
            aa, ra = inst(jnp.minimum(ta, n - 1))
            ab, rb = inst(jnp.clip(ta - 2, 0, n - 1))
            c = ((row0 + ac) * _COLS + rc) & (c_total - 1)
            g = gb_s[0, _shr(c, 7), c & 127]
            b = gb_s[1, _shr(c, 7), c & 127]
            n_s1 = _lanesum(p1)
            n_s2 = _lanesum(p2)
            mu = s1 * inv_n
            scale = g * lax.rsqrt(s2 * inv_n + _EPS)
            n_p2 = _pass_center(buf, ab, rb, mu, dbuf, (ta + 2) & 3)
            n_p1 = _pass_sum(buf, aa, ra)
            _pass_norm(buf, ac, rc, scale, b, dbuf, ta & 3)
            if head:
                rd_start(row0, ta + _AHEAD)
            return n_p1, n_s1, n_p2, n_s2

        nhead = n - _AHEAD
        carry = lax.fori_loop(0, nhead, lambda i, c: step(i, c, True), carry)
        for i in range(n - _FLIGHT, n - _RW):
            rd_wait(i)

        blocks = _write_blocks(nrows)
        for r in range(_EARLY):
            wr_column(row0, 0, blocks[0], r, wsem.at[0])
        for i in range(n - _RW, n):
            rd_wait(i)
        carry = lax.fori_loop(nhead, n + _PIPE, lambda i, c: step(i, c, False), carry)

        def columns(q0, q1, a_base, k, sem):
            def body(q, c):
                wr_column(row0, a_base + _shr(q, 3) * k, k, q & (_COLS - 1), sem)
                return c
            lax.fori_loop(q0, q1, body, 0)

        a_base, q0 = 0, _EARLY
        for k in sorted(set(blocks[:-1]), reverse=True):
            cnt = blocks[:-1].count(k)
            columns(q0, cnt * _COLS, a_base, k, wsem.at[0])
            a_base, q0 = a_base + cnt * k, 0
        kl = blocks[-1]
        columns(0, _COLS - 1, a_base, kl, wsem.at[1])
        last = [wr_copy(row0, a_base, kl, _COLS - 1, p, wsem.at[2 if p < 7 else 3])
                for p in range(8)]
        for cp in last:
            cp.start()
        v0 = buf.at[pl.ds(0, a_base)]
        pltpu.make_async_copy(v0, v0, wsem.at[0]).wait()
        v1 = buf.at[pl.ds(a_base, kl), pl.ds(0, _COLS - 1)]
        pltpu.make_async_copy(v1, v1, wsem.at[1]).wait()
        for cp in last[:-1]:
            cp.wait()
        if has_next:
            first_reads(row0 + nrows)
        last[-1].wait()
        if has_next:
            ramp(row0 + nrows)
        return carry

    carry = (gb_f[0],) * 4
    for row0 in range(0, rows_total, _CHUNK):
        nrows = min(_CHUNK, rows_total - row0)
        carry = chunk(row0, nrows, row0 + nrows < rows_total, carry)


@jax.jit
def pallas_standalone__instancenorm__prompt_kernel(
    x: jax.Array,
    g: jax.Array,
    b: jax.Array,
):
    bsz, c, h, w = x.shape
    rows = bsz * c // _COLS
    assert w == 32 and h % 1024 == 0 and h % _LC == 0 and c == 1024
    assert rows % _NA == 0 and (rows - 1) % _CHUNK + 1 >= 2 * _NA
    xt = jnp.transpose(x, (0, 1, 3, 2)).reshape(rows, _COLS, w, h)
    g2 = g.reshape(c // 128, 128)
    b2 = b.reshape(c // 128, 128)
    buf_bytes = (_CHUNK + 1) * _COLS * w * h * x.dtype.itemsize
    out = pl.pallas_call(
        _kernel,
        in_specs=[pl.BlockSpec(memory_space=pl.ANY)] * 3,
        out_specs=pl.BlockSpec(memory_space=pl.ANY),
        out_shape=jax.ShapeDtypeStruct(xt.shape, x.dtype),
        scratch_shapes=[
            pltpu.VMEM((_CHUNK + 1, _COLS, w, h), x.dtype),
            pltpu.VMEM((4, w, h), _F32),
            pltpu.VMEM((2, c // 128, 128), g.dtype),
            pltpu.VMEM((2, c // 128, 128), _F32),
            pltpu.SMEM((2, c // 128, 128), _F32),
            pltpu.SemaphoreType.DMA((_FLIGHT,)),
            pltpu.SemaphoreType.DMA((4,)),
        ],
        compiler_params=pltpu.CompilerParams(vmem_limit_bytes=buf_bytes + (8 << 20)),
    )(xt, g2, b2)
    return jnp.transpose(out.reshape(bsz, c, w, h), (0, 1, 3, 2))
```

```python
import jax
import jax.numpy as jnp
from jax import lax
import jax.experimental.pallas as pl
import jax.experimental.pallas.tpu as pltpu

_F32 = jnp.float32
_EPS = 1e-5

_COLS = 8
_NA = 16
_N0 = 2
_FLIGHT = 8
_AHEAD = _NA - 1 + _FLIGHT
_WK = 6
_EARLY = 5
_RW = 4
_WR = 4
_LC = 512
_PIPE = 4
_CHUNK = 96


def _shr(x, k):
    if isinstance(x, int):
        return x >> k
    return lax.shift_right_logical(x, jnp.int32(k))


def _ds(start, size, align):
    if isinstance(start, int):
        return pl.ds(start, size)
    return pl.ds(pl.multiple_of(start, align), size)


def _fold(v):
    parts = [v[:, l:l + 128] for l in range(0, v.shape[1], 128)]
    while len(parts) > 1:
        parts = [parts[i] + parts[i + 1] for i in range(0, len(parts), 2)]
    p = parts[0]
    p = p + pltpu.roll(p, 4, 0)
    p = p + pltpu.roll(p, 2, 0)
    p = p + pltpu.roll(p, 1, 0)
    return p


def _lanesum(p):
    return jnp.broadcast_to(jnp.sum(p, axis=1, keepdims=True), (8, 128))


def _slabs(buf):
    w, h = buf.shape[-2:]
    return [(pl.ds(q * 8, 8), pl.ds(l * _LC, _LC))
            for q in range(w // 8) for l in range(h // _LC)]


def _pass_sum(buf, a, r):
    acc = None
    for s, c in _slabs(buf):
        v = buf[a, r, s, c].astype(_F32)
        acc = v if acc is None else acc + v
    return _fold(acc)


def _pass_center(buf, a, r, mu, dbuf, k):
    acc = None
    m = jnp.tile(mu, (1, _LC // 128))
    for s, c in _slabs(buf):
        d = buf[a, r, s, c].astype(_F32) - m
        dbuf[k, s, c] = d
        d = d * d
        acc = d if acc is None else acc + d
    return _fold(acc)


def _pass_norm(buf, a, r, scale, beta, dbuf, k):
    sc = jnp.tile(scale, (1, _LC // 128))
    for s, c in _slabs(buf):
        buf[a, r, s, c] = (dbuf[k, s, c] * sc + beta).astype(buf.dtype)


def _last_block(nrows):
    a_last = (nrows // _WK - 1) * _WK
    return a_last, nrows - a_last


def _kernel(x_hbm, g_hbm, b_hbm, o_hbm, buf, dbuf, gb_v, gb_f, gb_s, fsem):
    def body(rsem, wsem):
        _body(x_hbm, g_hbm, b_hbm, o_hbm, buf, dbuf, gb_v, gb_f, gb_s, rsem, wsem, fsem)

    pl.run_scoped(body, pltpu.SemaphoreType.DMA((_FLIGHT,)), pltpu.SemaphoreType.DMA((4,)))
    a_last, kl = _last_block((x_hbm.shape[0] - 1) % _CHUNK + 1)
    v = buf.at[pl.ds(a_last, kl)]
    pltpu.make_async_copy(v, v, fsem).wait()


def _body(x_hbm, g_hbm, b_hbm, o_hbm, buf, dbuf, gb_v, gb_f, gb_s, rsem, wsem, fsem):
    rows_total, _, w, h = x_hbm.shape
    c_total = g_hbm.shape[0] * g_hbm.shape[1]
    inv_n = 1.0 / (w * h)
    dummy = buf.shape[0] - 1
    rl = h // 4

    def group(i):
        j = _shr(i, 4)
        return _shr(j, 3) * _NA, j & (_COLS - 1)

    def inst(i):
        a0, r = group(i)
        return a0 + (i & (_NA - 1)), r

    def rd_start(row0, i):
        a0, r = group(i)
        s = _ds((_shr(i, 2) & 3) * 8, 8, 8)
        sem = rsem.at[i & (_FLIGHT - 1)]
        for e, hi in ((0, True), (0, False), (1, False), (1, True)):
            c = _ds((i & 3) * rl + e * (rl // 2), rl // 2, 128)
            off, cnt = (0, _N0) if hi else (_N0, _NA - _N0)
            pltpu.make_async_copy(
                x_hbm.at[pl.ds(row0 + a0 + off, cnt), r, s, c],
                buf.at[pl.ds(a0 + off, cnt), r, s, c],
                sem).start(priority=0 if hi else 1)

    def rd_wait(i):
        a0, r = group(i)
        v = buf.at[pl.ds(a0, _NA), r,
                   _ds((_shr(i, 2) & 3) * 8, 8, 8), _ds((i & 3) * rl, rl, 128)]
        pltpu.make_async_copy(v, v, rsem.at[i & (_FLIGHT - 1)]).wait()

    def wr_copy(row0, a0, k, r, q, c, sem):
        s = _ds(q * 8, 8, 8)
        return pltpu.make_async_copy(
            buf.at[pl.ds(a0, k), r, s, c],
            o_hbm.at[pl.ds(row0 + a0, k), r, s, c], sem)

    def wr_strip(row0, a0, k, r, q, pieces, sem):
        wl = h // pieces
        return [wr_copy(row0, a0, k, r, q, pl.ds(p * wl, wl), sem) for p in range(pieces)]

    def wr_strips(row0, a0, k, i0, i1, sem):
        def body(i, c):
            for cp in wr_strip(row0, a0, k, _shr(i, 2), i & 3, 8, sem):
                cp.start()
            return c
        lax.fori_loop(i0, i1, body, 0)

    def wr_wait(v, sem):
        pltpu.make_async_copy(v, v, sem).wait()

    def first_reads(row0):
        for i in range(_FLIGHT):
            rd_start(row0, i)

    def ramp(row0):
        def body(i, c):
            rd_wait(i)
            rd_start(row0, i + _FLIGHT)
            return c
        lax.fori_loop(0, _NA - 1, body, 0)

    first_reads(0)

    cg = pltpu.make_async_copy(g_hbm, gb_v.at[0], wsem.at[0])
    cb = pltpu.make_async_copy(b_hbm, gb_v.at[1], wsem.at[1])
    cg.start()
    cb.start()
    dbuf[pl.ds(0, 2)] = jnp.zeros((2, w, h), _F32)
    cg.wait()
    cb.wait()
    gb_f[...] = gb_v[...].astype(_F32)
    cs = pltpu.make_async_copy(gb_f, gb_s, wsem.at[2])
    cs.start()
    ramp(0)
    cs.wait()

    def chunk(row0, nrows, has_next, carry):
        n = nrows * _COLS

        def step(ta, carry, head):
            p1, s1, p2, s2 = carry
            if head:
                rd_wait(ta + _NA - 1)
            t = ta - _PIPE
            ac, rc = inst(jnp.maximum(t, 0))
            ac = jnp.where(t >= 0, ac, dummy)
            aa, ra = inst(jnp.minimum(ta, n - 1))
            ab, rb = inst(jnp.clip(ta - 2, 0, n - 1))
            c = ((row0 + ac) * _COLS + rc) & (c_total - 1)
            g = gb_s[0, _shr(c, 7), c & 127]
            b = gb_s[1, _shr(c, 7), c & 127]
            n_s1 = _lanesum(p1)
            n_s2 = _lanesum(p2)
            mu = s1 * inv_n
            scale = g * lax.rsqrt(s2 * inv_n + _EPS)
            n_p2 = _pass_center(buf, ab, rb, mu, dbuf, (ta + 2) & 3)
            n_p1 = _pass_sum(buf, aa, ra)
            _pass_norm(buf, ac, rc, scale, b, dbuf, ta & 3)
            if head:
                rd_start(row0, ta + _AHEAD)
            return n_p1, n_s1, n_p2, n_s2

        nhead = n - _AHEAD
        carry = lax.fori_loop(0, nhead, lambda i, c: step(i, c, True), carry)
        for i in range(n - _FLIGHT, n - _RW):
            rd_wait(i)

        for i in range(4 * _EARLY):
            for cp in wr_strip(row0, 0, _WK, i >> 2, i & 3, 2, wsem.at[0]):
                cp.start()
        for i in range(n - _RW, n):
            rd_wait(i)
        carry = lax.fori_loop(nhead, n + _PIPE, lambda i, c: step(i, c, False), carry)
        wr_strips(row0, 0, _WK, 4 * _EARLY, 4 * _COLS, wsem.at[0])

        def block(j, c):
            wr_strips(row0, j * _WK, _WK, 0, 4 * _COLS, wsem.at[j & 1])
            wr_wait(buf.at[pl.ds((j - 1) * _WK, _WK)], wsem.at[(j - 1) & 1])
            return c

        a_last, kl = _last_block(nrows)
        jl = a_last // _WK
        lax.fori_loop(1, jl, block, 0)
        prev = buf.at[pl.ds(a_last - _WK, _WK)]
        if not has_next:
            wr_strips(row0, a_last, kl, 0, 4 * _COLS, fsem)
            wr_wait(prev, wsem.at[(jl - 1) & 1])
            return carry
        wr_strips(row0, a_last, kl, 0, 4 * (_COLS - 1), wsem.at[jl & 1])
        wr_strips(row0, a_last, kl, 4 * (_COLS - 1), 4 * _COLS - 1, wsem.at[2])
        last = [wr_copy(row0, a_last, kl, _COLS - 1, 3, pl.ds(p * (h // 8), h // 8),
                        fsem if p < 8 - _WR else wsem.at[3]) for p in range(8)]
        for cp in last:
            cp.start()
        wr_wait(prev, wsem.at[(jl - 1) & 1])
        wr_wait(buf.at[pl.ds(a_last, kl), pl.ds(0, _COLS - 1)], wsem.at[jl & 1])
        wr_wait(buf.at[pl.ds(a_last, kl), _COLS - 1, pl.ds(0, 24)], wsem.at[2])
        for cp in last[:8 - _WR]:
            cp.wait()
        first_reads(row0 + nrows)
        for cp in last[8 - _WR:]:
            cp.wait()
        ramp(row0 + nrows)
        return carry

    carry = (gb_f[0],) * 4
    for row0 in range(0, rows_total, _CHUNK):
        nrows = min(_CHUNK, rows_total - row0)
        carry = chunk(row0, nrows, row0 + nrows < rows_total, carry)


@jax.jit
def pallas_standalone__instancenorm__prompt_kernel(
    x: jax.Array,
    g: jax.Array,
    b: jax.Array,
):
    bsz, c, h, w = x.shape
    rows = bsz * c // _COLS
    assert w == 32 and h % 1024 == 0 and h % _LC == 0 and c == 1024
    assert rows % _NA == 0 and (rows - 1) % _CHUNK + 1 >= 2 * _NA
    xt = jnp.transpose(x, (0, 1, 3, 2)).reshape(rows, _COLS, w, h)
    g2 = g.reshape(c // 128, 128)
    b2 = b.reshape(c // 128, 128)
    buf_bytes = (_CHUNK + 1) * _COLS * w * h * x.dtype.itemsize
    out = pl.pallas_call(
        _kernel,
        in_specs=[pl.BlockSpec(memory_space=pl.ANY)] * 3,
        out_specs=pl.BlockSpec(memory_space=pl.ANY),
        out_shape=jax.ShapeDtypeStruct(xt.shape, x.dtype),
        scratch_shapes=[
            pltpu.VMEM((_CHUNK + 1, _COLS, w, h), x.dtype),
            pltpu.VMEM((4, w, h), _F32),
            pltpu.VMEM((2, c // 128, 128), g.dtype),
            pltpu.VMEM((2, c // 128, 128), _F32),
            pltpu.SMEM((2, c // 128, 128), _F32),
            pltpu.SemaphoreType.DMA(()),
        ],
        compiler_params=pltpu.CompilerParams(vmem_limit_bytes=buf_bytes + (8 << 20)),
    )(xt, g2, b2)
    return jnp.transpose(out.reshape(bsz, c, w, h), (0, 1, 3, 2))
```

```python
import jax
import jax.numpy as jnp
from jax import lax
import jax.experimental.pallas as pl
import jax.experimental.pallas.tpu as pltpu

_F32 = jnp.float32
_EPS = 1e-5

_COLS = 8
_NA = 16
_N0 = 2
_FLIGHT = 8
_AHEAD = _NA - 1 + _FLIGHT
_WK = 6
_EARLY = 5
_RW = 4
_WR = 4
_LC = 512
_PIPE = 4
_CHUNK = 96


def _shr(x, k):
    if isinstance(x, int):
        return x >> k
    return lax.shift_right_logical(x, jnp.int32(k))


def _ds(start, size, align):
    if isinstance(start, int):
        return pl.ds(start, size)
    return pl.ds(pl.multiple_of(start, align), size)


def _fold(v):
    parts = [v[:, l:l + 128] for l in range(0, v.shape[1], 128)]
    while len(parts) > 1:
        parts = [parts[i] + parts[i + 1] for i in range(0, len(parts), 2)]
    p = parts[0]
    p = p + pltpu.roll(p, 4, 0)
    p = p + pltpu.roll(p, 2, 0)
    p = p + pltpu.roll(p, 1, 0)
    return p


def _lanesum(p):
    return jnp.broadcast_to(jnp.sum(p, axis=1, keepdims=True), (8, 128))


def _slabs(buf):
    w, h = buf.shape[-2:]
    return [(pl.ds(q * 8, 8), pl.ds(l * _LC, _LC))
            for q in range(w // 8) for l in range(h // _LC)]


def _pass_sum(buf, a, r):
    acc = None
    for s, c in _slabs(buf):
        v = buf[a, r, s, c].astype(_F32)
        acc = v if acc is None else acc + v
    return _fold(acc)


def _pass_center(buf, a, r, mu, dbuf, k):
    acc = None
    m = jnp.tile(mu, (1, _LC // 128))
    for s, c in _slabs(buf):
        d = buf[a, r, s, c].astype(_F32) - m
        dbuf[k, s, c] = d
        d = d * d
        acc = d if acc is None else acc + d
    return _fold(acc)


def _pass_norm(buf, a, r, scale, beta, dbuf, k):
    sc = jnp.tile(scale, (1, _LC // 128))
    for s, c in _slabs(buf):
        buf[a, r, s, c] = (dbuf[k, s, c] * sc + beta).astype(buf.dtype)


def _last_block(nrows):
    a_last = (nrows // _WK - 1) * _WK
    return a_last, nrows - a_last


def _kernel(x_hbm, g_hbm, b_hbm, o_hbm, buf, dbuf, gb_v, gb_f, gb_s, fsem):
    def body(rsem, wsem):
        _body(x_hbm, g_hbm, b_hbm, o_hbm, buf, dbuf, gb_v, gb_f, gb_s, rsem, wsem, fsem)

    pl.run_scoped(body, pltpu.SemaphoreType.DMA((_FLIGHT,)), pltpu.SemaphoreType.DMA((4,)))
    a_last, kl = _last_block((x_hbm.shape[0] - 1) % _CHUNK + 1)
    v = buf.at[pl.ds(a_last, kl)]
    pltpu.make_async_copy(v, v, fsem).wait()


def _body(x_hbm, g_hbm, b_hbm, o_hbm, buf, dbuf, gb_v, gb_f, gb_s, rsem, wsem, fsem):
    rows_total, _, w, h = x_hbm.shape
    c_total = g_hbm.shape[0] * g_hbm.shape[1]
    inv_n = 1.0 / (w * h)
    dummy = buf.shape[0] - 1
    rl = h // 4

    def group(i):
        j = _shr(i, 4)
        return _shr(j, 3) * _NA, j & (_COLS - 1)

    def inst(i):
        a0, r = group(i)
        return a0 + (i & (_NA - 1)), r

    def rd_start(row0, i):
        a0, r = group(i)
        s = _ds((_shr(i, 2) & 3) * 8, 8, 8)
        sem = rsem.at[i & (_FLIGHT - 1)]
        for e, hi in ((0, True), (0, False), (1, False), (1, True)):
            c = _ds((i & 3) * rl + e * (rl // 2), rl // 2, 128)
            off, cnt = (0, _N0) if hi else (_N0, _NA - _N0)
            pltpu.make_async_copy(
                x_hbm.at[pl.ds(row0 + a0 + off, cnt), r, s, c],
                buf.at[pl.ds(a0 + off, cnt), r, s, c],
                sem).start(priority=0 if hi else 1)

    def rd_wait(i):
        a0, r = group(i)
        v = buf.at[pl.ds(a0, _NA), r,
                   _ds((_shr(i, 2) & 3) * 8, 8, 8), _ds((i & 3) * rl, rl, 128)]
        pltpu.make_async_copy(v, v, rsem.at[i & (_FLIGHT - 1)]).wait()

    def wr_copy(row0, a0, k, r, q, c, sem):
        s = _ds(q * 8, 8, 8)
        return pltpu.make_async_copy(
            buf.at[pl.ds(a0, k), r, s, c],
            o_hbm.at[pl.ds(row0 + a0, k), r, s, c], sem)

    def wr_strip(row0, a0, k, r, q, pieces, sem):
        wl = h // pieces
        return [wr_copy(row0, a0, k, r, q, pl.ds(p * wl, wl), sem) for p in range(pieces)]

    def wr_strips(row0, a0, k, i0, i1, sem):
        def body(i, c):
            for cp in wr_strip(row0, a0, k, _shr(i, 2), i & 3, 8, sem):
                cp.start()
            return c
        lax.fori_loop(i0, i1, body, 0)

    def wr_wait(v, sem):
        pltpu.make_async_copy(v, v, sem).wait()

    def first_reads(row0):
        for i in range(_FLIGHT):
            rd_start(row0, i)

    def ramp(row0):
        def body(i, c):
            rd_wait(i)
            rd_start(row0, i + _FLIGHT)
            return c
        lax.fori_loop(0, _NA - 1, body, 0)

    first_reads(0)

    cg = pltpu.make_async_copy(g_hbm, gb_v.at[0], wsem.at[0])
    cb = pltpu.make_async_copy(b_hbm, gb_v.at[1], wsem.at[1])
    cg.start()
    cb.start()
    dbuf[pl.ds(0, 2)] = jnp.zeros((2, w, h), _F32)
    cg.wait()
    cb.wait()
    gb_f[...] = gb_v[...].astype(_F32)
    cs = pltpu.make_async_copy(gb_f, gb_s, wsem.at[2])
    cs.start()
    ramp(0)
    cs.wait()

    def chunk(row0, nrows, has_next, carry):
        n = nrows * _COLS

        def step(ta, carry, head):
            (p1, s1, p2, s2), (ab, rb) = carry
            if head:
                rd_wait(ta + _NA - 1)
            t = ta - _PIPE
            ac, rc = inst(jnp.maximum(t, 0))
            ac = jnp.where(t >= 0, ac, dummy)
            aa, ra = inst(jnp.minimum(ta, n - 1))
            c = ((row0 + ac) * _COLS + rc) & (c_total - 1)
            g = gb_s[0, _shr(c, 7), c & 127]
            b = gb_s[1, _shr(c, 7), c & 127]
            n_s1 = _lanesum(p1)
            n_s2 = _lanesum(p2)
            mu = s1 * inv_n
            scale = g * lax.rsqrt(s2 * inv_n + _EPS)
            n_p2 = _pass_center(buf, ab, rb, mu, dbuf, (ta + 2) & 3)
            n_p1 = _pass_sum(buf, aa, ra)
            _pass_norm(buf, ac, rc, scale, b, dbuf, ta & 3)
            if head:
                rd_start(row0, ta + _AHEAD)
            return (n_p1, n_s1, n_p2, n_s2), inst(jnp.clip(ta - 1, 0, n - 1))

        nhead = n - _AHEAD
        carry = (carry, (jnp.int32(0), jnp.int32(0)))
        carry = lax.fori_loop(0, nhead, lambda i, c: step(i, c, True), carry)
        for i in range(n - _FLIGHT, n - _RW):
            rd_wait(i)

        for i in range(4 * _EARLY):
            for cp in wr_strip(row0, 0, _WK, i >> 2, i & 3, 2, wsem.at[0]):
                cp.start()
        for i in range(n - _RW, n):
            rd_wait(i)
        carry, _ = lax.fori_loop(nhead, n + _PIPE, lambda i, c: step(i, c, False), carry)
        wr_strips(row0, 0, _WK, 4 * _EARLY, 4 * _COLS, wsem.at[0])

        def block(j, c):
            wr_strips(row0, j * _WK, _WK, 0, 4 * _COLS, wsem.at[j & 1])
            wr_wait(buf.at[pl.ds((j - 1) * _WK, _WK)], wsem.at[(j - 1) & 1])
            return c

        a_last, kl = _last_block(nrows)
        jl = a_last // _WK
        lax.fori_loop(1, jl, block, 0)
        prev = buf.at[pl.ds(a_last - _WK, _WK)]
        if not has_next:
            wr_strips(row0, a_last, kl, 0, 4 * _COLS, fsem)
            wr_wait(prev, wsem.at[(jl - 1) & 1])
            return carry
        wr_strips(row0, a_last, kl, 0, 4 * (_COLS - 1), wsem.at[jl & 1])
        wr_strips(row0, a_last, kl, 4 * (_COLS - 1), 4 * _COLS - 1, wsem.at[2])
        last = [wr_copy(row0, a_last, kl, _COLS - 1, 3, pl.ds(p * (h // 8), h // 8),
                        fsem if p < 8 - _WR else wsem.at[3]) for p in range(8)]
        for cp in last:
            cp.start()
        wr_wait(prev, wsem.at[(jl - 1) & 1])
        wr_wait(buf.at[pl.ds(a_last, kl), pl.ds(0, _COLS - 1)], wsem.at[jl & 1])
        wr_wait(buf.at[pl.ds(a_last, kl), _COLS - 1, pl.ds(0, 24)], wsem.at[2])
        for cp in last[:8 - _WR]:
            cp.wait()
        first_reads(row0 + nrows)
        for cp in last[8 - _WR:]:
            cp.wait()
        ramp(row0 + nrows)
        return carry

    carry = (gb_f[0],) * 4
    for row0 in range(0, rows_total, _CHUNK):
        nrows = min(_CHUNK, rows_total - row0)
        carry = chunk(row0, nrows, row0 + nrows < rows_total, carry)


@jax.jit
def pallas_standalone__instancenorm__prompt_kernel(
    x: jax.Array,
    g: jax.Array,
    b: jax.Array,
):
    bsz, c, h, w = x.shape
    rows = bsz * c // _COLS
    assert w == 32 and h % 1024 == 0 and h % _LC == 0 and c == 1024
    assert rows % _NA == 0 and (rows - 1) % _CHUNK + 1 >= 2 * _NA
    xt = jnp.transpose(x, (0, 1, 3, 2)).reshape(rows, _COLS, w, h)
    g2 = g.reshape(c // 128, 128)
    b2 = b.reshape(c // 128, 128)
    buf_bytes = (_CHUNK + 1) * _COLS * w * h * x.dtype.itemsize
    out = pl.pallas_call(
        _kernel,
        in_specs=[pl.BlockSpec(memory_space=pl.ANY)] * 3,
        out_specs=pl.BlockSpec(memory_space=pl.ANY),
        out_shape=jax.ShapeDtypeStruct(xt.shape, x.dtype),
        scratch_shapes=[
            pltpu.VMEM((_CHUNK + 1, _COLS, w, h), x.dtype),
            pltpu.VMEM((4, w, h), _F32),
            pltpu.VMEM((2, c // 128, 128), g.dtype),
            pltpu.VMEM((2, c // 128, 128), _F32),
            pltpu.SMEM((2, c // 128, 128), _F32),
            pltpu.SemaphoreType.DMA(()),
        ],
        compiler_params=pltpu.CompilerParams(vmem_limit_bytes=buf_bytes + (8 << 20)),
    )(xt, g2, b2)
    return jnp.transpose(out.reshape(bsz, c, w, h), (0, 1, 3, 2))
```

```python
import jax
import jax.numpy as jnp
from jax import lax
import jax.experimental.pallas as pl
import jax.experimental.pallas.tpu as pltpu

_F32 = jnp.float32
_EPS = 1e-5

_COLS = 8
_NA = 16
_N0 = 2
_FLIGHT = 10
_RING = 16
_AHEAD = _NA - 1 + _FLIGHT
_WK = 6
_EARLY = 5
_RW = 4
_WR = 4
_LC = 512
_PIPE = 4
_CHUNK = 96


def _shr(x, k):
    if isinstance(x, int):
        return x >> k
    return lax.shift_right_logical(x, jnp.int32(k))


def _ds(start, size, align):
    if isinstance(start, int):
        return pl.ds(start, size)
    return pl.ds(pl.multiple_of(start, align), size)


def _fold(v):
    parts = [v[:, l:l + 128] for l in range(0, v.shape[1], 128)]
    while len(parts) > 1:
        parts = [parts[i] + parts[i + 1] for i in range(0, len(parts), 2)]
    p = parts[0]
    p = p + pltpu.roll(p, 4, 0)
    p = p + pltpu.roll(p, 2, 0)
    p = p + pltpu.roll(p, 1, 0)
    return p


def _lanesum(p):
    return jnp.broadcast_to(jnp.sum(p, axis=1, keepdims=True), (8, 128))


def _slabs(buf):
    w, h = buf.shape[-2:]
    return [(pl.ds(q * 8, 8), pl.ds(l * _LC, _LC))
            for q in range(w // 8) for l in range(h // _LC)]


def _pass_sum(buf, a, r):
    acc = None
    for s, c in _slabs(buf):
        v = buf[a, r, s, c].astype(_F32)
        acc = v if acc is None else acc + v
    return _fold(acc)


def _pass_center(buf, a, r, mu, dbuf, k):
    acc = None
    m = jnp.tile(mu, (1, _LC // 128))
    for s, c in _slabs(buf):
        d = buf[a, r, s, c].astype(_F32) - m
        dbuf[k, s, c] = d
        d = d * d
        acc = d if acc is None else acc + d
    return _fold(acc)


def _pass_norm(buf, a, r, scale, beta, dbuf, k):
    sc = jnp.tile(scale, (1, _LC // 128))
    for s, c in _slabs(buf):
        buf[a, r, s, c] = (dbuf[k, s, c] * sc + beta).astype(buf.dtype)


def _last_block(nrows):
    a_last = (nrows // _WK - 1) * _WK
    return a_last, nrows - a_last


def _kernel(x_hbm, g_hbm, b_hbm, o_hbm, buf, dbuf, gb_v, gb_f, gb_s, fsem):
    def body(rsem, wsem):
        _body(x_hbm, g_hbm, b_hbm, o_hbm, buf, dbuf, gb_v, gb_f, gb_s, rsem, wsem, fsem)

    pl.run_scoped(body, pltpu.SemaphoreType.DMA((_RING,)), pltpu.SemaphoreType.DMA((4,)))
    a_last, kl = _last_block((x_hbm.shape[0] - 1) % _CHUNK + 1)
    v = buf.at[pl.ds(a_last, kl)]
    pltpu.make_async_copy(v, v, fsem).wait()


def _body(x_hbm, g_hbm, b_hbm, o_hbm, buf, dbuf, gb_v, gb_f, gb_s, rsem, wsem, fsem):
    rows_total, _, w, h = x_hbm.shape
    c_total = g_hbm.shape[0] * g_hbm.shape[1]
    inv_n = 1.0 / (w * h)
    dummy = buf.shape[0] - 1
    rl = h // 4

    def group(i):
        j = _shr(i, 4)
        return _shr(j, 3) * _NA, j & (_COLS - 1)

    def inst(i):
        a0, r = group(i)
        return a0 + (i & (_NA - 1)), r

    def rd_start(row0, i):
        a0, r = group(i)
        s = _ds((_shr(i, 2) & 3) * 8, 8, 8)
        sem = rsem.at[i & (_RING - 1)]
        for e, hi in ((0, True), (0, False), (1, False), (1, True)):
            c = _ds((i & 3) * rl + e * (rl // 2), rl // 2, 128)
            off, cnt = (0, _N0) if hi else (_N0, _NA - _N0)
            pltpu.make_async_copy(
                x_hbm.at[pl.ds(row0 + a0 + off, cnt), r, s, c],
                buf.at[pl.ds(a0 + off, cnt), r, s, c],
                sem).start(priority=0 if hi else 1)

    def rd_wait(i):
        a0, r = group(i)
        v = buf.at[pl.ds(a0, _NA), r,
                   _ds((_shr(i, 2) & 3) * 8, 8, 8), _ds((i & 3) * rl, rl, 128)]
        pltpu.make_async_copy(v, v, rsem.at[i & (_RING - 1)]).wait()

    def wr_copy(row0, a0, k, r, q, c, sem):
        s = _ds(q * 8, 8, 8)
        return pltpu.make_async_copy(
            buf.at[pl.ds(a0, k), r, s, c],
            o_hbm.at[pl.ds(row0 + a0, k), r, s, c], sem)

    def wr_strip(row0, a0, k, r, q, pieces, sem):
        wl = h // pieces
        return [wr_copy(row0, a0, k, r, q, pl.ds(p * wl, wl), sem) for p in range(pieces)]

    def wr_strips(row0, a0, k, i0, i1, sem):
        def body(i, c):
            for cp in wr_strip(row0, a0, k, _shr(i, 2), i & 3, 8, sem):
                cp.start()
            return c
        lax.fori_loop(i0, i1, body, 0)

    def wr_wait(v, sem):
        pltpu.make_async_copy(v, v, sem).wait()

    def first_reads(row0):
        for i in range(_FLIGHT):
            rd_start(row0, i)

    def ramp(row0):
        def body(i, c):
            rd_wait(i)
            rd_start(row0, i + _FLIGHT)
            return c
        lax.fori_loop(0, _NA - 1, body, 0)

    first_reads(0)

    cg = pltpu.make_async_copy(g_hbm, gb_v.at[0], wsem.at[0])
    cb = pltpu.make_async_copy(b_hbm, gb_v.at[1], wsem.at[1])
    cg.start()
    cb.start()
    dbuf[pl.ds(0, 2)] = jnp.zeros((2, w, h), _F32)
    cg.wait()
    cb.wait()
    gb_f[...] = gb_v[...].astype(_F32)
    cs = pltpu.make_async_copy(gb_f, gb_s, wsem.at[2])
    cs.start()
    ramp(0)
    cs.wait()

    def chunk(row0, nrows, has_next, carry):
        n = nrows * _COLS

        def step(ta, carry, head):
            (p1, s1, p2, s2), (ab, rb) = carry
            if head:
                rd_wait(ta + _NA - 1)
            t = ta - _PIPE
            ac, rc = inst(jnp.maximum(t, 0))
            ac = jnp.where(t >= 0, ac, dummy)
            aa, ra = inst(jnp.minimum(ta, n - 1))
            c = ((row0 + ac) * _COLS + rc) & (c_total - 1)
            g = gb_s[0, _shr(c, 7), c & 127]
            b = gb_s[1, _shr(c, 7), c & 127]
            n_s1 = _lanesum(p1)
            n_s2 = _lanesum(p2)
            mu = s1 * inv_n
            scale = g * lax.rsqrt(s2 * inv_n + _EPS)
            n_p2 = _pass_center(buf, ab, rb, mu, dbuf, (ta + 2) & 3)
            n_p1 = _pass_sum(buf, aa, ra)
            _pass_norm(buf, ac, rc, scale, b, dbuf, ta & 3)
            if head:
                rd_start(row0, ta + _AHEAD)
            return (n_p1, n_s1, n_p2, n_s2), inst(jnp.clip(ta - 1, 0, n - 1))

        nhead = n - _AHEAD
        carry = (carry, (jnp.int32(0), jnp.int32(0)))
        carry = lax.fori_loop(0, nhead, lambda i, c: step(i, c, True), carry)
        for i in range(n - _FLIGHT, n - _RW):
            rd_wait(i)

        for i in range(4 * _EARLY):
            for cp in wr_strip(row0, 0, _WK, i >> 2, i & 3, 2, wsem.at[0]):
                cp.start()
        for i in range(n - _RW, n):
            rd_wait(i)
        carry, _ = lax.fori_loop(nhead, n + _PIPE, lambda i, c: step(i, c, False), carry)
        wr_strips(row0, 0, _WK, 4 * _EARLY, 4 * _COLS, wsem.at[0])

        def block(j, c):
            wr_strips(row0, j * _WK, _WK, 0, 4 * _COLS, wsem.at[j & 1])
            wr_wait(buf.at[pl.ds((j - 1) * _WK, _WK)], wsem.at[(j - 1) & 1])
            return c

        a_last, kl = _last_block(nrows)
        jl = a_last // _WK
        lax.fori_loop(1, jl, block, 0)
        prev = buf.at[pl.ds(a_last - _WK, _WK)]
        if not has_next:
            wr_strips(row0, a_last, kl, 0, 4 * _COLS, fsem)
            wr_wait(prev, wsem.at[(jl - 1) & 1])
            return carry
        wr_strips(row0, a_last, kl, 0, 4 * (_COLS - 1), wsem.at[jl & 1])
        wr_strips(row0, a_last, kl, 4 * (_COLS - 1), 4 * _COLS - 1, wsem.at[2])
        last = [wr_copy(row0, a_last, kl, _COLS - 1, 3, pl.ds(p * (h // 8), h // 8),
                        fsem if p < 8 - _WR else wsem.at[3]) for p in range(8)]
        for cp in last:
            cp.start()
        wr_wait(prev, wsem.at[(jl - 1) & 1])
        wr_wait(buf.at[pl.ds(a_last, kl), pl.ds(0, _COLS - 1)], wsem.at[jl & 1])
        wr_wait(buf.at[pl.ds(a_last, kl), _COLS - 1, pl.ds(0, 24)], wsem.at[2])
        for cp in last[:8 - _WR]:
            cp.wait()
        first_reads(row0 + nrows)
        for cp in last[8 - _WR:]:
            cp.wait()
        ramp(row0 + nrows)
        return carry

    carry = (gb_f[0],) * 4
    for row0 in range(0, rows_total, _CHUNK):
        nrows = min(_CHUNK, rows_total - row0)
        carry = chunk(row0, nrows, row0 + nrows < rows_total, carry)


@jax.jit
def pallas_standalone__instancenorm__prompt_kernel(
    x: jax.Array,
    g: jax.Array,
    b: jax.Array,
):
    bsz, c, h, w = x.shape
    rows = bsz * c // _COLS
    assert w == 32 and h % 1024 == 0 and h % _LC == 0 and c == 1024
    assert rows % _NA == 0 and (rows - 1) % _CHUNK + 1 >= 2 * _NA
    xt = jnp.transpose(x, (0, 1, 3, 2)).reshape(rows, _COLS, w, h)
    g2 = g.reshape(c // 128, 128)
    b2 = b.reshape(c // 128, 128)
    buf_bytes = (_CHUNK + 1) * _COLS * w * h * x.dtype.itemsize
    out = pl.pallas_call(
        _kernel,
        in_specs=[pl.BlockSpec(memory_space=pl.ANY)] * 3,
        out_specs=pl.BlockSpec(memory_space=pl.ANY),
        out_shape=jax.ShapeDtypeStruct(xt.shape, x.dtype),
        scratch_shapes=[
            pltpu.VMEM((_CHUNK + 1, _COLS, w, h), x.dtype),
            pltpu.VMEM((4, w, h), _F32),
            pltpu.VMEM((2, c // 128, 128), g.dtype),
            pltpu.VMEM((2, c // 128, 128), _F32),
            pltpu.SMEM((2, c // 128, 128), _F32),
            pltpu.SemaphoreType.DMA(()),
        ],
        compiler_params=pltpu.CompilerParams(vmem_limit_bytes=buf_bytes + (8 << 20)),
    )(xt, g2, b2)
    return jnp.transpose(out.reshape(bsz, c, w, h), (0, 1, 3, 2))
```

```python
import jax
import jax.numpy as jnp
from jax import lax
import jax.experimental.pallas as pl
import jax.experimental.pallas.tpu as pltpu

_F32 = jnp.float32
_EPS = 1e-5

_COLS = 8
_NA = 16
_N0 = 2
_FLIGHT = 10
_RING = 16
_AHEAD = _NA - 1 + _FLIGHT
_WK = 6
_EARLY = 5
_RW = 4
_WSPLIT = 7
_LC = 512
_PIPE = 4
_CHUNK = 96


def _shr(x, k):
    if isinstance(x, int):
        return x >> k
    return lax.shift_right_logical(x, jnp.int32(k))


def _ds(start, size, align):
    if isinstance(start, int):
        return pl.ds(start, size)
    return pl.ds(pl.multiple_of(start, align), size)


def _fold(v):
    parts = [v[:, l:l + 128] for l in range(0, v.shape[1], 128)]
    while len(parts) > 1:
        parts = [parts[i] + parts[i + 1] for i in range(0, len(parts), 2)]
    p = parts[0]
    p = p + pltpu.roll(p, 4, 0)
    p = p + pltpu.roll(p, 2, 0)
    p = p + pltpu.roll(p, 1, 0)
    return p


def _lanesum(p):
    return jnp.broadcast_to(jnp.sum(p, axis=1, keepdims=True), (8, 128))


def _slabs(buf):
    w, h = buf.shape[-2:]
    return [(pl.ds(q * 8, 8), pl.ds(l * _LC, _LC))
            for q in range(w // 8) for l in range(h // _LC)]


def _pass_sum(buf, a, r):
    acc = None
    for s, c in _slabs(buf):
        v = buf[a, r, s, c].astype(_F32)
        acc = v if acc is None else acc + v
    return _fold(acc)


def _pass_center(buf, a, r, mu, dbuf, k):
    acc = None
    m = jnp.tile(mu, (1, _LC // 128))
    for s, c in _slabs(buf):
        d = buf[a, r, s, c].astype(_F32) - m
        dbuf[k, s, c] = d
        d = d * d
        acc = d if acc is None else acc + d
    return _fold(acc)


def _pass_norm(buf, a, r, scale, beta, dbuf, k):
    sc = jnp.tile(scale, (1, _LC // 128))
    for s, c in _slabs(buf):
        buf[a, r, s, c] = (dbuf[k, s, c] * sc + beta).astype(buf.dtype)


def _last_block(nrows):
    a_last = (nrows // _WK - 1) * _WK
    return a_last, nrows - a_last


def _kernel(x_hbm, g_hbm, b_hbm, o_hbm, buf, dbuf, gb_v, gb_f, gb_s, fsem):
    def body(rsem, wsem):
        _body(x_hbm, g_hbm, b_hbm, o_hbm, buf, dbuf, gb_v, gb_f, gb_s, rsem, wsem, fsem)

    pl.run_scoped(body, pltpu.SemaphoreType.DMA((_RING,)), pltpu.SemaphoreType.DMA((4,)))
    a_last, kl = _last_block((x_hbm.shape[0] - 1) % _CHUNK + 1)
    v = buf.at[pl.ds(a_last, kl)]
    pltpu.make_async_copy(v, v, fsem).wait()


def _body(x_hbm, g_hbm, b_hbm, o_hbm, buf, dbuf, gb_v, gb_f, gb_s, rsem, wsem, fsem):
    rows_total, _, w, h = x_hbm.shape
    c_total = g_hbm.shape[0] * g_hbm.shape[1]
    inv_n = 1.0 / (w * h)
    dummy = buf.shape[0] - 1
    rl = h // 4

    def group(i):
        j = _shr(i, 4)
        return _shr(j, 3) * _NA, j & (_COLS - 1)

    def inst(i):
        a0, r = group(i)
        return a0 + (i & (_NA - 1)), r

    def rd_start(row0, i):
        a0, r = group(i)
        s = _ds((_shr(i, 2) & 3) * 8, 8, 8)
        sem = rsem.at[i & (_RING - 1)]
        for e, hi in ((0, True), (0, False), (1, False), (1, True)):
            c = _ds((i & 3) * rl + e * (rl // 2), rl // 2, 128)
            off, cnt = (0, _N0) if hi else (_N0, _NA - _N0)
            pltpu.make_async_copy(
                x_hbm.at[pl.ds(row0 + a0 + off, cnt), r, s, c],
                buf.at[pl.ds(a0 + off, cnt), r, s, c],
                sem).start(priority=0 if hi else 1)

    def rd_wait(i):
        a0, r = group(i)
        v = buf.at[pl.ds(a0, _NA), r,
                   _ds((_shr(i, 2) & 3) * 8, 8, 8), _ds((i & 3) * rl, rl, 128)]
        pltpu.make_async_copy(v, v, rsem.at[i & (_RING - 1)]).wait()

    def wr_strip(row0, a0, k, i, sems):
        r, s = _shr(i, 2), _ds((i & 3) * 8, 8, 8)
        cut = h // 16 * _WSPLIT
        return [pltpu.make_async_copy(buf.at[pl.ds(a0, k), r, s, c],
                                      o_hbm.at[pl.ds(row0 + a0, k), r, s, c], sem)
                for c, sem in zip((pl.ds(0, cut), pl.ds(cut, h - cut)), sems)]

    def wr_strips(row0, a0, k, i0, i1, sem):
        def body(i, c):
            for cp in wr_strip(row0, a0, k, i, (sem, sem)):
                cp.start()
            return c
        lax.fori_loop(i0, i1, body, 0)

    def wr_wait(v, sem):
        pltpu.make_async_copy(v, v, sem).wait()

    def first_reads(row0):
        for i in range(_FLIGHT):
            rd_start(row0, i)

    def ramp(row0):
        def body(i, c):
            rd_wait(i)
            rd_start(row0, i + _FLIGHT)
            return c
        lax.fori_loop(0, _NA - 1, body, 0)

    first_reads(0)

    cg = pltpu.make_async_copy(g_hbm, gb_v.at[0], wsem.at[0])
    cb = pltpu.make_async_copy(b_hbm, gb_v.at[1], wsem.at[1])
    cg.start()
    cb.start()
    dbuf[pl.ds(0, 2)] = jnp.zeros((2, w, h), _F32)
    cg.wait()
    cb.wait()
    gb_f[...] = gb_v[...].astype(_F32)
    cs = pltpu.make_async_copy(gb_f, gb_s, wsem.at[2])
    cs.start()
    ramp(0)
    cs.wait()

    def chunk(row0, nrows, has_next, carry):
        n = nrows * _COLS

        def step(ta, carry, head):
            (p1, s1, p2, s2), (ab, rb) = carry
            if head:
                rd_wait(ta + _NA - 1)
            t = ta - _PIPE
            ac, rc = inst(jnp.maximum(t, 0))
            ac = jnp.where(t >= 0, ac, dummy)
            aa, ra = inst(jnp.minimum(ta, n - 1))
            c = ((row0 + ac) * _COLS + rc) & (c_total - 1)
            g = gb_s[0, _shr(c, 7), c & 127]
            b = gb_s[1, _shr(c, 7), c & 127]
            n_s1 = _lanesum(p1)
            n_s2 = _lanesum(p2)
            mu = s1 * inv_n
            scale = g * lax.rsqrt(s2 * inv_n + _EPS)
            n_p2 = _pass_center(buf, ab, rb, mu, dbuf, (ta + 2) & 3)
            n_p1 = _pass_sum(buf, aa, ra)
            _pass_norm(buf, ac, rc, scale, b, dbuf, ta & 3)
            if head:
                rd_start(row0, ta + _AHEAD)
            return (n_p1, n_s1, n_p2, n_s2), inst(jnp.clip(ta - 1, 0, n - 1))

        nhead = n - _AHEAD
        carry = (carry, (jnp.int32(0), jnp.int32(0)))
        carry = lax.fori_loop(0, nhead, lambda i, c: step(i, c, True), carry)
        for i in range(n - _FLIGHT, n - _RW):
            rd_wait(i)

        wr_strips(row0, 0, _WK, 0, 4 * _EARLY, wsem.at[0])
        for i in range(n - _RW, n):
            rd_wait(i)
        carry, _ = lax.fori_loop(nhead, n + _PIPE, lambda i, c: step(i, c, False), carry)
        wr_strips(row0, 0, _WK, 4 * _EARLY, 4 * _COLS, wsem.at[0])

        def block(j, c):
            wr_strips(row0, j * _WK, _WK, 0, 4 * _COLS, wsem.at[j & 1])
            wr_wait(buf.at[pl.ds((j - 1) * _WK, _WK)], wsem.at[(j - 1) & 1])
            return c

        a_last, kl = _last_block(nrows)
        jl = a_last // _WK
        lax.fori_loop(1, jl, block, 0)
        prev = buf.at[pl.ds(a_last - _WK, _WK)]
        if not has_next:
            wr_strips(row0, a_last, kl, 0, 4 * _COLS, fsem)
            wr_wait(prev, wsem.at[(jl - 1) & 1])
            return carry
        wr_strips(row0, a_last, kl, 0, 4 * (_COLS - 1), wsem.at[jl & 1])
        wr_strips(row0, a_last, kl, 4 * (_COLS - 1), 4 * _COLS - 1, wsem.at[2])
        last = wr_strip(row0, a_last, kl, 4 * _COLS - 1, (fsem, wsem.at[3]))
        for cp in last:
            cp.start()
        wr_wait(prev, wsem.at[(jl - 1) & 1])
        wr_wait(buf.at[pl.ds(a_last, kl), pl.ds(0, _COLS - 1)], wsem.at[jl & 1])
        wr_wait(buf.at[pl.ds(a_last, kl), _COLS - 1, pl.ds(0, 24)], wsem.at[2])
        last[0].wait()
        first_reads(row0 + nrows)
        last[1].wait()
        ramp(row0 + nrows)
        return carry

    carry = (gb_f[0],) * 4
    for row0 in range(0, rows_total, _CHUNK):
        nrows = min(_CHUNK, rows_total - row0)
        carry = chunk(row0, nrows, row0 + nrows < rows_total, carry)


@jax.jit
def pallas_standalone__instancenorm__prompt_kernel(
    x: jax.Array,
    g: jax.Array,
    b: jax.Array,
):
    bsz, c, h, w = x.shape
    rows = bsz * c // _COLS
    assert w == 32 and h % 2048 == 0 and h % _LC == 0 and c == 1024
    assert rows % _NA == 0 and (rows - 1) % _CHUNK + 1 >= 2 * _NA
    xt = jnp.transpose(x, (0, 1, 3, 2)).reshape(rows, _COLS, w, h)
    g2 = g.reshape(c // 128, 128)
    b2 = b.reshape(c // 128, 128)
    buf_bytes = (_CHUNK + 1) * _COLS * w * h * x.dtype.itemsize
    out = pl.pallas_call(
        _kernel,
        in_specs=[pl.BlockSpec(memory_space=pl.ANY)] * 3,
        out_specs=pl.BlockSpec(memory_space=pl.ANY),
        out_shape=jax.ShapeDtypeStruct(xt.shape, x.dtype),
        scratch_shapes=[
            pltpu.VMEM((_CHUNK + 1, _COLS, w, h), x.dtype),
            pltpu.VMEM((4, w, h), _F32),
            pltpu.VMEM((2, c // 128, 128), g.dtype),
            pltpu.VMEM((2, c // 128, 128), _F32),
            pltpu.SMEM((2, c // 128, 128), _F32),
            pltpu.SemaphoreType.DMA(()),
        ],
        compiler_params=pltpu.CompilerParams(vmem_limit_bytes=buf_bytes + (8 << 20)),
    )(xt, g2, b2)
    return jnp.transpose(out.reshape(bsz, c, w, h), (0, 1, 3, 2))
```

```python
import jax
import jax.numpy as jnp
from jax import lax
import jax.experimental.pallas as pl
import jax.experimental.pallas.tpu as pltpu

_F32 = jnp.float32
_EPS = 1e-5

_COLS = 8
_NA = 16
_N0 = 2
_FLIGHT = 10
_RING = 16
_AHEAD = _NA - 1 + _FLIGHT
_WK = 6
_EARLY = 5
_RW = 4
_WSPLIT = 7
_LC = 512
_PIPE = 4
_CHUNK = 96


def _shr(x, k):
    if isinstance(x, int):
        return x >> k
    return lax.shift_right_logical(x, jnp.int32(k))


def _ds(start, size, align):
    if isinstance(start, int):
        return pl.ds(start, size)
    return pl.ds(pl.multiple_of(start, align), size)


def _fold(v):
    parts = [v[:, l:l + 128] for l in range(0, v.shape[1], 128)]
    while len(parts) > 1:
        parts = [parts[i] + parts[i + 1] for i in range(0, len(parts), 2)]
    p = parts[0]
    p = p + pltpu.roll(p, 4, 0)
    p = p + pltpu.roll(p, 2, 0)
    p = p + pltpu.roll(p, 1, 0)
    return p


def _lanesum(p):
    return jnp.broadcast_to(jnp.sum(p, axis=1, keepdims=True), (8, 128))


def _slabs(buf):
    w, h = buf.shape[-2:]
    return [(pl.ds(q * 8, 8), pl.ds(l * _LC, _LC))
            for q in range(w // 8) for l in range(h // _LC)]


def _pass_sum(buf, a, r):
    acc = None
    for s, c in _slabs(buf):
        v = buf[a, r, s, c].astype(_F32)
        acc = v if acc is None else acc + v
    return _fold(acc)


def _pass_center(buf, a, r, mu, dbuf, k):
    acc = None
    m = jnp.tile(mu, (1, _LC // 128))
    for s, c in _slabs(buf):
        d = buf[a, r, s, c].astype(_F32) - m
        dbuf[k, s, c] = d
        d = d * d
        acc = d if acc is None else acc + d
    return _fold(acc)


def _pass_norm(buf, a, r, scale, beta, dbuf, k):
    sc = jnp.tile(scale, (1, _LC // 128))
    for s, c in _slabs(buf):
        buf[a, r, s, c] = (dbuf[k, s, c] * sc + beta).astype(buf.dtype)


def _last_block(nrows):
    a_last = (nrows // _WK - 1) * _WK
    return a_last, nrows - a_last


def _kernel(x_hbm, g_hbm, b_hbm, o_hbm, buf, dbuf, gb_v, gb_f, gb_s, fsem):
    def body(rsem, wsem):
        _body(x_hbm, g_hbm, b_hbm, o_hbm, buf, dbuf, gb_v, gb_f, gb_s, rsem, wsem, fsem)

    pl.run_scoped(body, pltpu.SemaphoreType.DMA((_RING,)), pltpu.SemaphoreType.DMA((4,)))
    a_last, kl = _last_block((x_hbm.shape[0] - 1) % _CHUNK + 1)
    v = buf.at[pl.ds(a_last, kl)]
    pltpu.make_async_copy(v, v, fsem).wait()


def _body(x_hbm, g_hbm, b_hbm, o_hbm, buf, dbuf, gb_v, gb_f, gb_s, rsem, wsem, fsem):
    rows_total, _, w, h = x_hbm.shape
    c_total = g_hbm.shape[0] * g_hbm.shape[1]
    inv_n = 1.0 / (w * h)
    dummy = buf.shape[0] - 1
    rl = h // 4

    def group(i):
        j = _shr(i, 4)
        return _shr(j, 3) * _NA, j & (_COLS - 1)

    def inst(i):
        a0, r = group(i)
        return a0 + (i & (_NA - 1)), r

    def rd_start(row0, i):
        a0, r = group(i)
        s = _ds((_shr(i, 2) & 3) * 8, 8, 8)
        sem = rsem.at[i & (_RING - 1)]
        for e, hi in ((0, True), (0, False), (1, False), (1, True)):
            c = _ds((i & 3) * rl + e * (rl // 2), rl // 2, 128)
            off, cnt = (0, _N0) if hi else (_N0, _NA - _N0)
            pltpu.make_async_copy(
                x_hbm.at[pl.ds(row0 + a0 + off, cnt), r, s, c],
                buf.at[pl.ds(a0 + off, cnt), r, s, c],
                sem).start(priority=0 if hi else 1)

    def rd_wait(i):
        a0, r = group(i)
        v = buf.at[pl.ds(a0, _NA), r,
                   _ds((_shr(i, 2) & 3) * 8, 8, 8), _ds((i & 3) * rl, rl, 128)]
        pltpu.make_async_copy(v, v, rsem.at[i & (_RING - 1)]).wait()

    def wr_strip(row0, a0, k, i, sems):
        r, s = _shr(i, 2), _ds((i & 3) * 8, 8, 8)
        cut = h // 16 * _WSPLIT
        return [pltpu.make_async_copy(buf.at[pl.ds(a0, k), r, s, c],
                                      o_hbm.at[pl.ds(row0 + a0, k), r, s, c], sem)
                for c, sem in zip((pl.ds(0, cut), pl.ds(cut, h - cut)), sems)]

    def wr_strips(row0, a0, k, i0, i1, sem):
        def body(i, c):
            for cp in wr_strip(row0, a0, k, i, (sem, sem)):
                cp.start()
            return c
        lax.fori_loop(i0, i1, body, 0)

    def wr_wait(v, sem):
        pltpu.make_async_copy(v, v, sem).wait()

    def first_reads(row0):
        def body(i, c):
            rd_start(row0, i)
            return c
        lax.fori_loop(0, _FLIGHT, body, 0)

    def ramp(row0):
        def body(i, c):
            rd_wait(i)
            rd_start(row0, i + _FLIGHT)
            return c
        lax.fori_loop(0, _NA - 1, body, 0)

    first_reads(0)

    cg = pltpu.make_async_copy(g_hbm, gb_v.at[0], wsem.at[0])
    cb = pltpu.make_async_copy(b_hbm, gb_v.at[1], wsem.at[1])
    cg.start()
    cb.start()
    dbuf[pl.ds(0, 2)] = jnp.zeros((2, w, h), _F32)
    cg.wait()
    cb.wait()
    gb_f[...] = gb_v[...].astype(_F32)
    cs = pltpu.make_async_copy(gb_f, gb_s, wsem.at[2])
    cs.start()
    ramp(0)
    cs.wait()

    nfull = (rows_total - 1) // _CHUNK
    rows_last = rows_total - nfull * _CHUNK

    def chunk(ci, carry):
        row0 = ci * _CHUNK
        has_next = ci < nfull
        n = jnp.where(has_next, _CHUNK, rows_last) * _COLS

        def step(ta, carry, head):
            (p1, s1, p2, s2), (ab, rb) = carry
            if head:
                rd_wait(ta + _NA - 1)
            t = ta - _PIPE
            ac, rc = inst(jnp.maximum(t, 0))
            ac = jnp.where(t >= 0, ac, dummy)
            aa, ra = inst(jnp.minimum(ta, n - 1))
            c = ((row0 + ac) * _COLS + rc) & (c_total - 1)
            g = gb_s[0, _shr(c, 7), c & 127]
            b = gb_s[1, _shr(c, 7), c & 127]
            n_s1 = _lanesum(p1)
            n_s2 = _lanesum(p2)
            mu = s1 * inv_n
            scale = g * lax.rsqrt(s2 * inv_n + _EPS)
            n_p2 = _pass_center(buf, ab, rb, mu, dbuf, (ta + 2) & 3)
            n_p1 = _pass_sum(buf, aa, ra)
            _pass_norm(buf, ac, rc, scale, b, dbuf, ta & 3)
            if head:
                rd_start(row0, ta + _AHEAD)
            return (n_p1, n_s1, n_p2, n_s2), inst(jnp.clip(ta - 1, 0, n - 1))

        nhead = n - _AHEAD
        carry = (carry, (jnp.int32(0), jnp.int32(0)))
        carry = lax.fori_loop(0, nhead, lambda i, c: step(i, c, True), carry)
        for i in range(-_FLIGHT, -_RW):
            rd_wait(n + i)

        wr_strips(row0, 0, _WK, 0, 4 * _EARLY, wsem.at[0])
        for i in range(-_RW, 0):
            rd_wait(n + i)
        carry, _ = lax.fori_loop(nhead, n + _PIPE, lambda i, c: step(i, c, False), carry)
        wr_strips(row0, 0, _WK, 4 * _EARLY, 4 * _COLS, wsem.at[0])

        def block(j, c):
            wr_strips(row0, j * _WK, _WK, 0, 4 * _COLS, wsem.at[j & 1])
            wr_wait(buf.at[pl.ds((j - 1) * _WK, _WK)], wsem.at[(j - 1) & 1])
            return c

        lax.fori_loop(1, jnp.where(has_next, _CHUNK // _WK, rows_last // _WK) - 1, block, 0)

        @pl.when(has_next)
        def _():
            a_last, kl = _last_block(_CHUNK)
            jl = a_last // _WK
            wr_strips(row0, a_last, kl, 0, 4 * (_COLS - 1), wsem.at[jl & 1])
            wr_strips(row0, a_last, kl, 4 * (_COLS - 1), 4 * _COLS - 1, wsem.at[2])
            last = wr_strip(row0, a_last, kl, 4 * _COLS - 1, (fsem, wsem.at[3]))
            for cp in last:
                cp.start()
            wr_wait(buf.at[pl.ds(a_last - _WK, _WK)], wsem.at[(jl - 1) & 1])
            wr_wait(buf.at[pl.ds(a_last, kl), pl.ds(0, _COLS - 1)], wsem.at[jl & 1])
            wr_wait(buf.at[pl.ds(a_last, kl), _COLS - 1, pl.ds(0, 24)], wsem.at[2])
            last[0].wait()
            first_reads(row0 + _CHUNK)
            last[1].wait()
            ramp(row0 + _CHUNK)

        return carry

    carry = (gb_f[0],) * 4
    lax.fori_loop(0, nfull + 1, chunk, carry)
    a_last, kl = _last_block(rows_last)
    wr_strips(nfull * _CHUNK, a_last, kl, 0, 4 * _COLS, fsem)
    wr_wait(buf.at[pl.ds(a_last - _WK, _WK)], wsem.at[(a_last // _WK - 1) & 1])


@jax.jit
def pallas_standalone__instancenorm__prompt_kernel(
    x: jax.Array,
    g: jax.Array,
    b: jax.Array,
):
    bsz, c, h, w = x.shape
    rows = bsz * c // _COLS
    assert w == 32 and h % 2048 == 0 and h % _LC == 0 and c == 1024
    assert rows % _NA == 0 and (rows - 1) % _CHUNK + 1 >= 2 * _NA
    xt = jnp.transpose(x, (0, 1, 3, 2)).reshape(rows, _COLS, w, h)
    g2 = g.reshape(c // 128, 128)
    b2 = b.reshape(c // 128, 128)
    buf_bytes = (_CHUNK + 1) * _COLS * w * h * x.dtype.itemsize
    out = pl.pallas_call(
        _kernel,
        in_specs=[pl.BlockSpec(memory_space=pl.ANY)] * 3,
        out_specs=pl.BlockSpec(memory_space=pl.ANY),
        out_shape=jax.ShapeDtypeStruct(xt.shape, x.dtype),
        scratch_shapes=[
            pltpu.VMEM((_CHUNK + 1, _COLS, w, h), x.dtype),
            pltpu.VMEM((4, w, h), _F32),
            pltpu.VMEM((2, c // 128, 128), g.dtype),
            pltpu.VMEM((2, c // 128, 128), _F32),
            pltpu.SMEM((2, c // 128, 128), _F32),
            pltpu.SemaphoreType.DMA(()),
        ],
        compiler_params=pltpu.CompilerParams(vmem_limit_bytes=buf_bytes + (8 << 20)),
    )(xt, g2, b2)
    return jnp.transpose(out.reshape(bsz, c, w, h), (0, 1, 3, 2))
```

```python
import jax
import jax.numpy as jnp
from jax import lax
import jax.experimental.pallas as pl
import jax.experimental.pallas.tpu as pltpu

_F32 = jnp.float32
_EPS = 1e-5

_COLS = 8
_NA = 16
_N0 = 2
_FLIGHT = 10
_RING = 16
_AHEAD = _NA - 1 + _FLIGHT
_WK = 6
_EARLY = 5
_RW = 4
_COARSE = (7, 9)
_FINE = (2, 1, 2, 1, 2, 2, 1, 2, 1, 2)
_LC = 512
_PIPE = 4
_CHUNK = 96


def _shr(x, k):
    if isinstance(x, int):
        return x >> k
    return lax.shift_right_logical(x, jnp.int32(k))


def _ds(start, size, align):
    if isinstance(start, int):
        return pl.ds(start, size)
    return pl.ds(pl.multiple_of(start, align), size)


def _fold(v):
    parts = [v[:, l:l + 128] for l in range(0, v.shape[1], 128)]
    while len(parts) > 1:
        parts = [parts[i] + parts[i + 1] for i in range(0, len(parts), 2)]
    p = parts[0]
    p = p + pltpu.roll(p, 4, 0)
    p = p + pltpu.roll(p, 2, 0)
    p = p + pltpu.roll(p, 1, 0)
    return p


def _lanesum(p):
    return jnp.broadcast_to(jnp.sum(p, axis=1, keepdims=True), (8, 128))


def _slabs(buf):
    w, h = buf.shape[-2:]
    return [(pl.ds(q * 8, 8), pl.ds(l * _LC, _LC))
            for q in range(w // 8) for l in range(h // _LC)]


def _pass_sum(buf, a, r):
    acc = None
    for s, c in _slabs(buf):
        v = buf[a, r, s, c].astype(_F32)
        acc = v if acc is None else acc + v
    return _fold(acc)


def _pass_center(buf, a, r, mu, dbuf, k):
    acc = None
    m = jnp.tile(mu, (1, _LC // 128))
    for s, c in _slabs(buf):
        d = buf[a, r, s, c].astype(_F32) - m
        dbuf[k, s, c] = d
        d = d * d
        acc = d if acc is None else acc + d
    return _fold(acc)


def _pass_norm(buf, a, r, scale, beta, dbuf, k):
    sc = jnp.tile(scale, (1, _LC // 128))
    for s, c in _slabs(buf):
        buf[a, r, s, c] = (dbuf[k, s, c] * sc + beta).astype(buf.dtype)


def _last_block(nrows):
    a_last = (nrows // _WK - 1) * _WK
    return a_last, nrows - a_last


def _kernel(x_hbm, g_hbm, b_hbm, o_hbm, buf, dbuf, gb_v, gb_f, gb_s, fsem):
    def body(rsem, wsem):
        _body(x_hbm, g_hbm, b_hbm, o_hbm, buf, dbuf, gb_v, gb_f, gb_s, rsem, wsem, fsem)

    pl.run_scoped(body, pltpu.SemaphoreType.DMA((_RING,)), pltpu.SemaphoreType.DMA((4,)))
    a_last, kl = _last_block((x_hbm.shape[0] - 1) % _CHUNK + 1)
    v = buf.at[pl.ds(a_last, kl)]
    pltpu.make_async_copy(v, v, fsem).wait()


def _body(x_hbm, g_hbm, b_hbm, o_hbm, buf, dbuf, gb_v, gb_f, gb_s, rsem, wsem, fsem):
    rows_total, _, w, h = x_hbm.shape
    c_total = g_hbm.shape[0] * g_hbm.shape[1]
    inv_n = 1.0 / (w * h)
    dummy = buf.shape[0] - 1
    rl = h // 4

    def group(i):
        j = _shr(i, 4)
        return _shr(j, 3) * _NA, j & (_COLS - 1)

    def inst(i):
        a0, r = group(i)
        return a0 + (i & (_NA - 1)), r

    def rd_start(row0, i):
        a0, r = group(i)
        s = _ds((_shr(i, 2) & 3) * 8, 8, 8)
        sem = rsem.at[i & (_RING - 1)]
        for e, hi in ((0, True), (0, False), (1, False), (1, True)):
            c = _ds((i & 3) * rl + e * (rl // 2), rl // 2, 128)
            off, cnt = (0, _N0) if hi else (_N0, _NA - _N0)
            pltpu.make_async_copy(
                x_hbm.at[pl.ds(row0 + a0 + off, cnt), r, s, c],
                buf.at[pl.ds(a0 + off, cnt), r, s, c],
                sem).start(priority=0 if hi else 1)

    def rd_wait(i):
        a0, r = group(i)
        v = buf.at[pl.ds(a0, _NA), r,
                   _ds((_shr(i, 2) & 3) * 8, 8, 8), _ds((i & 3) * rl, rl, 128)]
        pltpu.make_async_copy(v, v, rsem.at[i & (_RING - 1)]).wait()

    def wr_strip(row0, a0, k, i, cuts, sems):
        r, s = _shr(i, 2), _ds((i & 3) * 8, 8, 8)
        lanes = [pl.ds(sum(cuts[:p]) * (h // 16), cuts[p] * (h // 16)) for p in range(len(cuts))]
        return [pltpu.make_async_copy(buf.at[pl.ds(a0, k), r, s, c],
                                      o_hbm.at[pl.ds(row0 + a0, k), r, s, c], sem)
                for c, sem in zip(lanes, sems)]

    def wr_strips(row0, a0, k, i0, i1, sem, cuts=_FINE):
        def body(i, c):
            for cp in wr_strip(row0, a0, k, i, cuts, [sem] * len(cuts)):
                cp.start()
            return c
        lax.fori_loop(i0, i1, body, 0)

    def wr_wait(v, sem):
        pltpu.make_async_copy(v, v, sem).wait()

    def first_reads(row0):
        def body(i, c):
            rd_start(row0, i)
            return c
        lax.fori_loop(0, _FLIGHT, body, 0)

    def ramp(row0):
        def body(i, c):
            rd_wait(i)
            rd_start(row0, i + _FLIGHT)
            return c
        lax.fori_loop(0, _NA - 1, body, 0)

    first_reads(0)

    cg = pltpu.make_async_copy(g_hbm, gb_v.at[0], wsem.at[0])
    cb = pltpu.make_async_copy(b_hbm, gb_v.at[1], wsem.at[1])
    cg.start()
    cb.start()
    dbuf[pl.ds(0, 2)] = jnp.zeros((2, w, h), _F32)
    cg.wait()
    cb.wait()
    gb_f[...] = gb_v[...].astype(_F32)
    cs = pltpu.make_async_copy(gb_f, gb_s, wsem.at[2])
    cs.start()
    ramp(0)
    cs.wait()

    nfull = (rows_total - 1) // _CHUNK
    rows_last = rows_total - nfull * _CHUNK

    def chunk(ci, carry):
        row0 = ci * _CHUNK
        has_next = ci < nfull
        n = jnp.where(has_next, _CHUNK, rows_last) * _COLS

        def step(ta, carry, head):
            (p1, s1, p2, s2), (ab, rb) = carry
            if head:
                rd_wait(ta + _NA - 1)
            t = ta - _PIPE
            ac, rc = inst(jnp.maximum(t, 0))
            ac = jnp.where(t >= 0, ac, dummy)
            aa, ra = inst(jnp.minimum(ta, n - 1))
            c = ((row0 + ac) * _COLS + rc) & (c_total - 1)
            g = gb_s[0, _shr(c, 7), c & 127]
            b = gb_s[1, _shr(c, 7), c & 127]
            n_s1 = _lanesum(p1)
            n_s2 = _lanesum(p2)
            mu = s1 * inv_n
            scale = g * lax.rsqrt(s2 * inv_n + _EPS)
            n_p2 = _pass_center(buf, ab, rb, mu, dbuf, (ta + 2) & 3)
            n_p1 = _pass_sum(buf, aa, ra)
            _pass_norm(buf, ac, rc, scale, b, dbuf, ta & 3)
            if head:
                rd_start(row0, ta + _AHEAD)
            return (n_p1, n_s1, n_p2, n_s2), inst(jnp.clip(ta - 1, 0, n - 1))

        nhead = n - _AHEAD
        carry = (carry, (jnp.int32(0), jnp.int32(0)))
        carry = lax.fori_loop(0, nhead, lambda i, c: step(i, c, True), carry)
        for i in range(-_FLIGHT, -_RW):
            rd_wait(n + i)

        wr_strips(row0, 0, _WK, 0, 4 * _EARLY, wsem.at[0], _COARSE)
        for i in range(-_RW, 0):
            rd_wait(n + i)
        carry, _ = lax.fori_loop(nhead, n + _PIPE, lambda i, c: step(i, c, False), carry)
        wr_strips(row0, 0, _WK, 4 * _EARLY, 4 * _COLS, wsem.at[0])

        def block(j, c):
            wr_strips(row0, j * _WK, _WK, 0, 4 * _COLS, wsem.at[j & 1])
            wr_wait(buf.at[pl.ds((j - 1) * _WK, _WK)], wsem.at[(j - 1) & 1])
            return c

        lax.fori_loop(1, jnp.where(has_next, _CHUNK // _WK, rows_last // _WK) - 1, block, 0)

        @pl.when(has_next)
        def _():
            a_last, kl = _last_block(_CHUNK)
            jl = a_last // _WK
            wr_strips(row0, a_last, kl, 0, 4 * (_COLS - 1), wsem.at[jl & 1])
            wr_strips(row0, a_last, kl, 4 * (_COLS - 1), 4 * _COLS - 1, wsem.at[2])
            last = wr_strip(row0, a_last, kl, 4 * _COLS - 1, _COARSE, (fsem, wsem.at[3]))
            for cp in last:
                cp.start()
            wr_wait(buf.at[pl.ds(a_last - _WK, _WK)], wsem.at[(jl - 1) & 1])
            wr_wait(buf.at[pl.ds(a_last, kl), pl.ds(0, _COLS - 1)], wsem.at[jl & 1])
            wr_wait(buf.at[pl.ds(a_last, kl), _COLS - 1, pl.ds(0, 24)], wsem.at[2])
            last[0].wait()
            first_reads(row0 + _CHUNK)
            last[1].wait()
            ramp(row0 + _CHUNK)

        return carry

    carry = (gb_f[0],) * 4
    lax.fori_loop(0, nfull + 1, chunk, carry)
    a_last, kl = _last_block(rows_last)
    wr_strips(nfull * _CHUNK, a_last, kl, 0, 4 * _COLS, fsem)
    wr_wait(buf.at[pl.ds(a_last - _WK, _WK)], wsem.at[(a_last // _WK - 1) & 1])


@jax.jit
def pallas_standalone__instancenorm__prompt_kernel(
    x: jax.Array,
    g: jax.Array,
    b: jax.Array,
):
    bsz, c, h, w = x.shape
    rows = bsz * c // _COLS
    assert w == 32 and h % 2048 == 0 and h % _LC == 0 and c == 1024
    assert rows % _NA == 0 and (rows - 1) % _CHUNK + 1 >= 2 * _NA
    xt = jnp.transpose(x, (0, 1, 3, 2)).reshape(rows, _COLS, w, h)
    g2 = g.reshape(c // 128, 128)
    b2 = b.reshape(c // 128, 128)
    buf_bytes = (_CHUNK + 1) * _COLS * w * h * x.dtype.itemsize
    out = pl.pallas_call(
        _kernel,
        in_specs=[pl.BlockSpec(memory_space=pl.ANY)] * 3,
        out_specs=pl.BlockSpec(memory_space=pl.ANY),
        out_shape=jax.ShapeDtypeStruct(xt.shape, x.dtype),
        scratch_shapes=[
            pltpu.VMEM((_CHUNK + 1, _COLS, w, h), x.dtype),
            pltpu.VMEM((4, w, h), _F32),
            pltpu.VMEM((2, c // 128, 128), g.dtype),
            pltpu.VMEM((2, c // 128, 128), _F32),
            pltpu.SMEM((2, c // 128, 128), _F32),
            pltpu.SemaphoreType.DMA(()),
        ],
        compiler_params=pltpu.CompilerParams(vmem_limit_bytes=buf_bytes + (8 << 20)),
    )(xt, g2, b2)
    return jnp.transpose(out.reshape(bsz, c, w, h), (0, 1, 3, 2))
```

```python
import jax
import jax.numpy as jnp
from jax import lax
import jax.experimental.pallas as pl
import jax.experimental.pallas.tpu as pltpu

_F32 = jnp.float32
_EPS = 1e-5

_COLS = 8
_NA = 16
_N0 = 2
_FLIGHT = 10
_RING = 16
_AHEAD = _NA - 1 + _FLIGHT
_WK = 6
_EARLY = 5
_RW = 4
_COARSE = (7, 9)
_FINE = (2, 1, 2, 1, 2, 2, 1, 2, 1, 2)
_LC = 512
_PIPE = 4
_CHUNK = 96


def _shr(x, k):
    if isinstance(x, int):
        return x >> k
    return lax.shift_right_logical(x, jnp.int32(k))


def _ds(start, size, align):
    if isinstance(start, int):
        return pl.ds(start, size)
    return pl.ds(pl.multiple_of(start, align), size)


def _fold(v):
    parts = [v[:, l:l + 128] for l in range(0, v.shape[1], 128)]
    while len(parts) > 1:
        parts = [parts[i] + parts[i + 1] for i in range(0, len(parts), 2)]
    p = parts[0]
    p = p + pltpu.roll(p, 4, 0)
    p = p + pltpu.roll(p, 2, 0)
    p = p + pltpu.roll(p, 1, 0)
    return p


def _lanesum(p):
    return jnp.broadcast_to(jnp.sum(p, axis=1, keepdims=True), (8, 128))


def _slabs(buf):
    w, h = buf.shape[-2:]
    return [(pl.ds(q * 8, 8), pl.ds(l * _LC, _LC))
            for q in range(w // 8) for l in range(h // _LC)]


def _pass_sum(buf, a, r):
    acc = None
    for s, c in _slabs(buf):
        v = buf[a, r, s, c].astype(_F32)
        acc = v if acc is None else acc + v
    return _fold(acc)


def _pass_center(buf, a, r, mu, dbuf, k):
    acc = None
    m = jnp.tile(mu, (1, _LC // 128))
    for s, c in _slabs(buf):
        d = buf[a, r, s, c].astype(_F32) - m
        dbuf[k, s, c] = d
        d = d * d
        acc = d if acc is None else acc + d
    return _fold(acc)


def _pass_norm(buf, a, r, scale, beta, dbuf, k):
    sc = jnp.tile(scale, (1, _LC // 128))
    for s, c in _slabs(buf):
        buf[a, r, s, c] = (dbuf[k, s, c] * sc + beta).astype(buf.dtype)


def _last_block(nrows):
    a_last = (nrows // _WK - 1) * _WK
    return a_last, nrows - a_last


def _kernel(x_hbm, g_hbm, b_hbm, o_hbm, buf, dbuf, gb_v, gb_f, gb_s, fsem):
    def body(rsem, wsem):
        _body(x_hbm, g_hbm, b_hbm, o_hbm, buf, dbuf, gb_v, gb_f, gb_s, rsem, wsem, fsem)

    pl.run_scoped(body, pltpu.SemaphoreType.DMA((_RING,)), pltpu.SemaphoreType.DMA((4,)))
    a_last, kl = _last_block((x_hbm.shape[0] - 1) % _CHUNK + 1)
    pltpu.make_async_copy(buf.at[pl.ds(a_last, kl)],
                          o_hbm.at[pl.ds(o_hbm.shape[0] - kl, kl)], fsem).wait()


def _body(x_hbm, g_hbm, b_hbm, o_hbm, buf, dbuf, gb_v, gb_f, gb_s, rsem, wsem, fsem):
    rows_total, _, w, h = x_hbm.shape
    c_total = g_hbm.shape[0] * g_hbm.shape[1]
    inv_n = 1.0 / (w * h)
    dummy = buf.shape[0] - 1
    rl = h // 4

    def group(i):
        j = _shr(i, 4)
        return _shr(j, 3) * _NA, j & (_COLS - 1)

    def inst(i):
        a0, r = group(i)
        return a0 + (i & (_NA - 1)), r

    def rd_start(row0, i):
        a0, r = group(i)
        s = _ds((_shr(i, 2) & 3) * 8, 8, 8)
        sem = rsem.at[i & (_RING - 1)]
        for e, hi in ((0, True), (0, False), (1, False), (1, True)):
            c = _ds((i & 3) * rl + e * (rl // 2), rl // 2, 128)
            off, cnt = (0, _N0) if hi else (_N0, _NA - _N0)
            pltpu.make_async_copy(
                x_hbm.at[pl.ds(row0 + a0 + off, cnt), r, s, c],
                buf.at[pl.ds(a0 + off, cnt), r, s, c],
                sem).start(priority=0 if hi else 1)

    def rd_wait(i):
        a0, r = group(i)
        v = buf.at[pl.ds(a0, _NA), r,
                   _ds((_shr(i, 2) & 3) * 8, 8, 8), _ds((i & 3) * rl, rl, 128)]
        pltpu.make_async_copy(v, v, rsem.at[i & (_RING - 1)]).wait()

    def wr_strip(row0, a0, k, i, cuts, sems):
        r, s = _shr(i, 2), _ds((i & 3) * 8, 8, 8)
        lanes = [pl.ds(sum(cuts[:p]) * (h // 16), cuts[p] * (h // 16)) for p in range(len(cuts))]
        return [pltpu.make_async_copy(buf.at[pl.ds(a0, k), r, s, c],
                                      o_hbm.at[pl.ds(row0 + a0, k), r, s, c], sem)
                for c, sem in zip(lanes, sems)]

    def wr_strips(row0, a0, k, i0, i1, sem, cuts=_FINE):
        def body(i, c):
            for cp in wr_strip(row0, a0, k, i, cuts, [sem] * len(cuts)):
                cp.start()
            return c
        lax.fori_loop(i0, i1, body, 0)

    def wr_wait(row0, a0, k, sem, *idx):
        pltpu.make_async_copy(buf.at[(pl.ds(a0, k),) + idx],
                              o_hbm.at[(pl.ds(row0 + a0, k),) + idx], sem).wait()

    def first_reads(row0):
        def body(i, c):
            rd_start(row0, i)
            return c
        lax.fori_loop(0, _FLIGHT, body, 0)

    def ramp(row0):
        def body(i, c):
            rd_wait(i)
            rd_start(row0, i + _FLIGHT)
            return c
        lax.fori_loop(0, _NA - 1, body, 0)

    first_reads(0)

    cg = pltpu.make_async_copy(g_hbm, gb_v.at[0], wsem.at[0])
    cb = pltpu.make_async_copy(b_hbm, gb_v.at[1], wsem.at[1])
    cg.start()
    cb.start()
    dbuf[pl.ds(0, 2)] = jnp.zeros((2, w, h), _F32)
    cg.wait()
    cb.wait()
    gb_f[...] = gb_v[...].astype(_F32)
    cs = pltpu.make_async_copy(gb_f, gb_s, wsem.at[2])
    cs.start()
    ramp(0)
    cs.wait()

    nfull = (rows_total - 1) // _CHUNK
    rows_last = rows_total - nfull * _CHUNK

    def chunk(ci, carry):
        row0 = ci * _CHUNK
        has_next = ci < nfull
        n = jnp.where(has_next, _CHUNK, rows_last) * _COLS

        def step(ta, carry, head):
            (p1, s1, p2, s2), (ab, rb) = carry
            if head:
                rd_wait(ta + _NA - 1)
            t = ta - _PIPE
            ac, rc = inst(jnp.maximum(t, 0))
            ac = jnp.where(t >= 0, ac, dummy)
            aa, ra = inst(jnp.minimum(ta, n - 1))
            c = ((row0 + ac) * _COLS + rc) & (c_total - 1)
            g = gb_s[0, _shr(c, 7), c & 127]
            b = gb_s[1, _shr(c, 7), c & 127]
            n_s1 = _lanesum(p1)
            n_s2 = _lanesum(p2)
            mu = s1 * inv_n
            scale = g * lax.rsqrt(s2 * inv_n + _EPS)
            n_p2 = _pass_center(buf, ab, rb, mu, dbuf, (ta + 2) & 3)
            n_p1 = _pass_sum(buf, aa, ra)
            _pass_norm(buf, ac, rc, scale, b, dbuf, ta & 3)
            if head:
                rd_start(row0, ta + _AHEAD)
            return (n_p1, n_s1, n_p2, n_s2), inst(jnp.clip(ta - 1, 0, n - 1))

        nhead = n - _AHEAD
        carry = (carry, (jnp.int32(0), jnp.int32(0)))
        carry = lax.fori_loop(0, nhead, lambda i, c: step(i, c, True), carry)
        for i in range(-_FLIGHT, -_RW):
            rd_wait(n + i)

        wr_strips(row0, 0, _WK, 0, 4 * _EARLY, wsem.at[0], _COARSE)
        for i in range(-_RW, 0):
            rd_wait(n + i)
        carry, _ = lax.fori_loop(nhead, n + _PIPE, lambda i, c: step(i, c, False), carry)
        wr_strips(row0, 0, _WK, 4 * _EARLY, 4 * _COLS, wsem.at[0])

        def block(j, c):
            wr_strips(row0, j * _WK, _WK, 0, 4 * _COLS, wsem.at[j & 1])
            wr_wait(row0, (j - 1) * _WK, _WK, wsem.at[(j - 1) & 1])
            return c

        lax.fori_loop(1, jnp.where(has_next, _CHUNK // _WK, rows_last // _WK) - 1, block, 0)

        @pl.when(has_next)
        def _():
            a_last, kl = _last_block(_CHUNK)
            jl = a_last // _WK
            wr_strips(row0, a_last, kl, 0, 4 * (_COLS - 1), wsem.at[jl & 1])
            wr_strips(row0, a_last, kl, 4 * (_COLS - 1), 4 * _COLS - 1, wsem.at[2])
            last = wr_strip(row0, a_last, kl, 4 * _COLS - 1, _COARSE, (fsem, wsem.at[3]))
            for cp in last:
                cp.start()
            wr_wait(row0, a_last - _WK, _WK, wsem.at[(jl - 1) & 1])
            wr_wait(row0, a_last, kl, wsem.at[jl & 1], pl.ds(0, _COLS - 1))
            wr_wait(row0, a_last, kl, wsem.at[2], _COLS - 1, pl.ds(0, 24))
            last[0].wait()
            first_reads(row0 + _CHUNK)
            last[1].wait()
            ramp(row0 + _CHUNK)

        return carry

    carry = (gb_f[0],) * 4
    lax.fori_loop(0, nfull + 1, chunk, carry)
    a_last, kl = _last_block(rows_last)
    wr_strips(nfull * _CHUNK, a_last, kl, 0, 4 * _COLS, fsem)
    wr_wait(nfull * _CHUNK, a_last - _WK, _WK, wsem.at[(a_last // _WK - 1) & 1])


@jax.jit
def pallas_standalone__instancenorm__prompt_kernel(
    x: jax.Array,
    g: jax.Array,
    b: jax.Array,
):
    bsz, c, h, w = x.shape
    rows = bsz * c // _COLS
    assert w == 32 and h % 2048 == 0 and h % _LC == 0 and c == 1024
    assert rows % _NA == 0 and (rows - 1) % _CHUNK + 1 >= 2 * _NA
    xt = jnp.transpose(x, (0, 1, 3, 2)).reshape(rows, _COLS, w, h)
    g2 = g.reshape(c // 128, 128)
    b2 = b.reshape(c // 128, 128)
    buf_bytes = (_CHUNK + 1) * _COLS * w * h * x.dtype.itemsize
    out = pl.pallas_call(
        _kernel,
        in_specs=[pl.BlockSpec(memory_space=pl.ANY)] * 3,
        out_specs=pl.BlockSpec(memory_space=pl.ANY),
        out_shape=jax.ShapeDtypeStruct(xt.shape, x.dtype),
        scratch_shapes=[
            pltpu.VMEM((_CHUNK + 1, _COLS, w, h), x.dtype),
            pltpu.VMEM((4, w, h), _F32),
            pltpu.VMEM((2, c // 128, 128), g.dtype),
            pltpu.VMEM((2, c // 128, 128), _F32),
            pltpu.SMEM((2, c // 128, 128), _F32),
            pltpu.SemaphoreType.DMA(()),
        ],
        compiler_params=pltpu.CompilerParams(vmem_limit_bytes=buf_bytes + (8 << 20)),
    )(xt, g2, b2)
    return jnp.transpose(out.reshape(bsz, c, w, h), (0, 1, 3, 2))
```
